```python
import jax
import jax.numpy as jnp

def _softmax(x, axis=-1):
    return jax.nn.softmax(x, axis=axis)

def _gelu(x):
    return jax.nn.gelu(x, approximate=True)

def _silu(x):
    return jax.nn.silu(x)

def _sigmoid(x):
    return jax.nn.sigmoid(x)

def _layernorm(x, axis=-1, eps=1e-05):
    m = jnp.mean(x, axis=axis, keepdims=True)
    v = jnp.var(x, axis=axis, keepdims=True)
    return (x - m) / jnp.sqrt(v + eps)

def _scatter_add(tgt, idx, src, axis=0):
    return tgt.at[idx].add(src)

def _segment_sum(src, seg, n):
    return jax.ops.segment_sum(src, seg, n)

class _Rng:

    def __init__(self, key):
        self._k = key

    def _next(self):
        self._k, sub = jax.random.split(self._k)
        return sub

    def normal(self, shape):
        return jax.random.normal(self._next(), shape, dtype=jnp.bfloat16)

    def randint(self, lo, hi, shape):
        return jax.random.randint(self._next(), shape, lo, hi, dtype=jnp.int32)

    def uniform(self, shape, lo=0.0, hi=1.0):
        return jax.random.uniform(self._next(), shape, jnp.bfloat16, lo, hi)

    def permutation(self, n):
        return jax.random.permutation(self._next(), n)
kernel_name = 'concat_heads__memory_aug_recurrent_mem_tr__ssm_conv_h3__prompt'

def setup_inputs():
    _rng = _Rng(jax.random.key(int.from_bytes(__import__("os").urandom(4), "little")))
    _w = lambda a: (lambda t: t.astype(jnp.bfloat16) if jnp.issubdtype(t.dtype, jnp.floating) else t)(jnp.asarray(a))

    def _A_setup():
        B, S, Dm = (1, 2048, 1024)
        H, Dh = (32, 128)
        M, seg = (8, 32)
        seg = min(seg, S)
        S = S // seg * seg
        return {'x': _w((lambda *s: _rng.normal(s) * 0.05)(B, S, Dm)), 'mem0': _w((lambda *s: _rng.normal(s) * 0.05)(B, M, Dm)), 'Wq': _w((lambda *s: _rng.normal(s) * 0.05)(Dm, H, Dh) * Dm ** (-0.5)), 'Wk': _w((lambda *s: _rng.normal(s) * 0.05)(Dm, H, Dh) * Dm ** (-0.5)), 'Wv': _w((lambda *s: _rng.normal(s) * 0.05)(Dm, H, Dh) * Dm ** (-0.5)), 'Wo': _w((lambda *s: _rng.normal(s) * 0.05)(H, Dh, Dm) * (H * Dh) ** (-0.5)), 'seg_len': seg}
    _A_in = _A_setup()

    def _B_setup():
        B, S, D = (1, 2048, 1024)
        ks = 4
        return {'q': _w((lambda *s: _rng.normal(s) * 0.05)(B, S, D)), 'k': _w((lambda *s: _rng.normal(s) * 0.05)(B, S, D)), 'v': _w((lambda *s: _rng.normal(s) * 0.05)(B, S, D)), 'shift_k': _w((lambda *s: _rng.normal(s) * 0.05)(D, ks) * 0.5), 'ssm_k': _w((lambda *s: _rng.normal(s) * 0.05)(D, S) * (1.0 / S ** 0.5)), 'ssm_D': _w((lambda *s: _rng.normal(s) * 0.05)(D))}
    _B_in = _B_setup()
    return {'A_x': _A_in['x'], 'A_mem0': _A_in['mem0'], 'A_Wq': _A_in['Wq'], 'A_Wk': _A_in['Wk'], 'A_Wv': _A_in['Wv'], 'A_Wo': _A_in['Wo'], 'A_seg_len': _A_in['seg_len'], 'B_q': _B_in['q'], 'B_k': _B_in['k'], 'B_v': _B_in['v'], 'B_shift_k': _B_in['shift_k'], 'B_ssm_k': _B_in['ssm_k'], 'B_ssm_D': _B_in['ssm_D']}

def reference(A_x, A_mem0, A_Wq, A_Wk, A_Wv, A_Wo, A_seg_len, B_q, B_k, B_v, B_shift_k, B_ssm_k, B_ssm_D):

    def _A_ref(x, mem0, Wq, Wk, Wv, Wo, seg_len):
        B, S, Dm = x.shape
        H, Dh = (Wq.shape[1], Wq.shape[2])
        M = mem0.shape[1]
        scale = Dh ** (-0.5)
        n_seg = S // seg_len
        L = M + seg_len
        idx = jnp.arange(L)
        mask = (idx[:, None] < M) | (idx[:, None] >= idx[None, :])
        mem = mem0
        outs = []
        for s in range(n_seg):
            xs = x[:, s * seg_len:(s + 1) * seg_len, :].copy()
            h = jnp.concatenate([mem, xs], axis=1)
            q = jnp.einsum('btd,dhe->bhte', h, Wq)
            k = jnp.einsum('btd,dhe->bhte', h, Wk)
            v = jnp.einsum('btd,dhe->bhte', h, Wv)
            scores = jnp.einsum('bhqe,bhke->bhqk', q, k) * scale
            scores = jnp.where(mask[None, None], scores, -1000000000.0)
            p = _softmax(scores, axis=-1)
            o = jnp.einsum('bhqk,bhke->bhqe', p, v)
            o = jnp.einsum('bhte,hed->btd', o, Wo)
            mem = o[:, :M, :].copy()
            outs.append(o[:, M:, :])
        return jnp.concatenate(outs, axis=1)

    def _B_ref(q, k, v, shift_k, ssm_k, ssm_D):
        B, S, D = q.shape
        ks = shift_k.shape[-1]
        k_pad = jnp.pad(k, ((0, 0), (ks - 1, 0), (0, 0)))
        k_shift = jnp.zeros_like(k)
        for t in range(ks):
            k_shift = k_shift + k_pad[:, t:t + S, :] * shift_k[:, ks - 1 - t][None, None, :]
        kv = k_shift * v
        L = 2 * S
        kv_pad = jnp.pad(kv, ((0, 0), (0, S), (0, 0)))
        kf_pad = jnp.pad(ssm_k, ((0, 0), (0, S)))
        kv_f = (lambda x, axes=(-2, -1): jnp.fft.rfft2(x.astype(jnp.float32), axes=axes))(kv_pad[:, None, :, :], axes=(1, 2))
        kf_f = (lambda x, axes=(-2, -1): jnp.fft.rfft2(x.astype(jnp.float32), axes=axes))(kf_pad[:, None, :], axes=(1, 2))
        kf_f = (lambda x, *d: x.transpose(*d))(kf_f, 1, 2, 0)
        y_f = kv_f * kf_f[None, :, :, :]
        y = (lambda x, s, axes=(-2, -1): jnp.fft.irfft2(x, s=s, axes=axes).astype(jnp.bfloat16))(y_f, (1, L), axes=(1, 2))[:, 0, :S, :]
        y = y + kv * ssm_D[None, None, :]
        return q * y
    a = _A_ref(A_x, A_mem0, A_Wq, A_Wk, A_Wv, A_Wo, A_seg_len)
    b = _B_ref(B_q, B_k, B_v, B_shift_k, B_ssm_k, B_ssm_D)
    return jnp.concatenate([a, b], axis=-1)
```

```python
import functools
import jax, jax.numpy as jnp, numpy as np
from jax.experimental import pallas as pl
from jax.experimental.pallas import tpu as pltpu

S, DM, H, DH, M, SEG = 2048, 1024, 32, 128, 8, 32
D = 1024
NSEG = S // SEG
L = M + SEG
NT = (((1,), (1,)), ((), ()))
NN = (((1,), (0,)), ((), ()))
def _dot(a, b, dims=NN):
    return jax.lax.dot_general(a, b, dims, preferred_element_type=jnp.float32)

def dft_consts():
    N = 256; C = 128
    f_order = np.concatenate([np.arange(0, 128, 2), np.arange(1, 128, 2)])
    th = 2 * np.pi * np.outer(f_order + 0.5, np.arange(C)) / N
    F = np.concatenate([np.cos(th), -np.sin(th)], 0)
    G = np.concatenate([np.cos(th).T, -np.sin(th).T], 1) * (2.0 / N)
    return F.astype(np.float32), G.astype(np.float32)

def make(GB=4, order="mid2", doB=True):
    scale = DH ** -0.5
    def kern(x_hbm, mem0_ref, wq_hbm, wk_hbm, wv_hbm, wo_hbm,
             q_hbm, k_hbm, v_hbm, sk_ref, w_hbm, dd_ref, f_ref, g_ref, out_hbm,
             xv, raw, wqkv, wo32, osta, sems, osema,
             kin, vin, win, qin, kf32, kvb, uh, whp, wprev, skt, ybuf, ost, isem, qsem, osem):
        def in_copies(j, p):
            c = pl.multiple_of(j * 128, 128)
            return [pltpu.make_async_copy(k_hbm.at[:, pl.ds(c, 128)], kin.at[p], isem.at[p, 0]),
                    pltpu.make_async_copy(v_hbm.at[:, pl.ds(c, 128)], vin.at[p], isem.at[p, 1]),
                    pltpu.make_async_copy(w_hbm.at[pl.ds(c, 128), :], win.at[p], isem.at[p, 2])]
        def q_copy(j, p):
            c = pl.multiple_of(j * 128, 128)
            return pltpu.make_async_copy(q_hbm.at[:, pl.ds(c, 128)], qin.at[p], qsem.at[p])
        def out_copy(j, a, slot):
            return pltpu.make_async_copy(ost.at[slot], out_hbm.at[pl.ds(pl.multiple_of(a * 128, 128), 128), pl.ds(pl.multiple_of(D + j * 128, 128), 128)], osem.at[slot])
        def outa_copy(s, slot):
            return pltpu.make_async_copy(osta.at[slot], out_hbm.at[pl.ds(pl.multiple_of(s * SEG, SEG), SEG), pl.ds(0, DM)], osema.at[slot])

        for cp in in_copies(0, 0): cp.start()
        cpx = pltpu.make_async_copy(x_hbm, xv, sems.at[0]); cpx.start()
        skt[0:4, :] = sk_ref[...].astype(jnp.float32).T
        skt[4:5, :] = dd_ref[...].astype(jnp.float32)
        kf32[0:8, :] = jnp.zeros((8, 128), jnp.float32)
        F = f_ref[...]; G = g_ref[...]

        def stage1(j, p, i):
            r0 = pl.multiple_of(i * 256, 256)
            c0 = pl.multiple_of(j * 128, 128)
            taps = skt[:, pl.ds(c0, 128)]
            kf = kin[p, pl.ds(r0, 256), :].astype(jnp.float32)
            kf32[pl.ds(r0 + 8, 256), :] = kf
            ks = (kf * taps[0:1] + kf32[pl.ds(r0 + 7, 256), :] * taps[1:2]
                  + kf32[pl.ds(r0 + 6, 256), :] * taps[2:3] + kf32[pl.ds(r0 + 5, 256), :] * taps[3:4])
            kv = ks * vin[p, pl.ds(r0, 256), :].astype(jnp.float32)
            kvb[p, pl.ds(r0, 256), :] = kv
            prev = jnp.where(i == 0, 0.0, wprev[...])
            for c in range(2):
                a = 2 * i + c
                uh[p, a] = _dot(F, kv[c * 128:(c + 1) * 128])
                wt = win[p, :, pl.ds(pl.multiple_of(a * 128, 128), 128)]
                wh = _dot(F, wt, NT)
                pr, pi_ = prev[:128], prev[128:]
                re = jnp.concatenate([wh[0:64] - pi_[0:64], wh[64:128] + pi_[64:128]], 0)
                im = jnp.concatenate([wh[128:192] + pr[0:64], wh[192:256] - pr[64:128]], 0)
                whp[p, a, 0:128] = re
                whp[p, a, 128:256] = im
                prev = wh
            wprev[...] = prev

        def stage2(j, p, i, par):
            c0 = pl.multiple_of(j * 128, 128)
            dvec = skt[4:5, pl.ds(c0, 128)]
            ms = [jnp.where(n <= i, n, n - i - 1) for n in range(17)]
            aus = [jnp.where(n <= i, i - n, 16 - n) for n in range(17)]
            dst = [jnp.where(n == i, 0, 1) for n in range(17)]
            tot = []
            for gb in range(16 // GB):
                accr = [None] * GB; acci = [None] * GB
                for n in range(17):
                    for gg in range(GB):
                        g = gb * GB + gg
                        ur = uh[p, aus[n], 8 * g:8 * g + 8, :]; ui = uh[p, aus[n], 128 + 8 * g:128 + 8 * g + 8, :]
                        wr = whp[p, ms[n], 8 * g:8 * g + 8, :]; wi = whp[p, ms[n], 128 + 8 * g:128 + 8 * g + 8, :]
                        tr = ur * wr - ui * wi; ti = ur * wi + ui * wr
                        accr[gg] = tr if n == 0 else accr[gg] + tr
                        acci[gg] = ti if n == 0 else acci[gg] + ti
                        if n < 8:
                            ybuf[dst[n], 8 * g:8 * g + 8, :] = accr[gg]
                            ybuf[dst[n], 128 + 8 * g:128 + 8 * g + 8, :] = acci[gg]
                tot.append((accr, acci))
            totr = jnp.concatenate([t for (ar, ai) in tot for t in ar], 0)
            toti = jnp.concatenate([t for (ar, ai) in tot for t in ai], 0)
            y1 = ybuf[0]
            y2 = jnp.concatenate([totr, toti], 0) - y1
            for sl, (a, Y) in enumerate(((i, y1), (15 - i, y2))):
                y = _dot(G, Y)
                r = pl.multiple_of(a * 128, 128)
                o = qin[p, pl.ds(r, 128), :].astype(jnp.float32) * (y + kvb[p, pl.ds(r, 128), :] * dvec)
                ost[par * 2 + sl] = o.astype(jnp.bfloat16)

        for j, w_hbm_ in enumerate((wq_hbm, wk_hbm, wv_hbm)):
            cp = pltpu.make_async_copy(w_hbm_, raw.bitcast(jnp.bfloat16), sems.at[1])
            cp.start(); cp.wait()
            def per_hp(hp, c, j=j):
                for jj in range(8):
                    for t in range(8):
                        d0 = jj * 128 + t * 16
                        A = raw[pl.ds(d0 * 16 + hp, 8, stride=32), :]
                        B = raw[pl.ds(d0 * 16 + 16 + hp, 8, stride=32), :]
                        o0 = (A & jnp.uint32(0xFFFF)) | (B << 16)
                        o1 = (A >> 16) | (B & jnp.uint32(0xFFFF0000))
                        c0 = pl.multiple_of((2 * hp) * 384 + j * 128, 128)
                        c1 = pl.multiple_of((2 * hp + 1) * 384 + j * 128, 128)
                        wqkv[pl.ds(d0 // 2, 8), pl.ds(c0, 128)] = o0
                        wqkv[pl.ds(d0 // 2, 8), pl.ds(c1, 128)] = o1
                return c
            jax.lax.fori_loop(0, 16, per_hp, 0)
        cp = pltpu.make_async_copy(wo_hbm, wo32.bitcast(jnp.bfloat16), sems.at[1])
        cp.start()
        for cq in in_copies(1, 1): cq.start()
        q_copy(0, 0).start()
        for cq in in_copies(0, 0): cq.wait()
        def pro(i, c):
            stage1(0, 0, i); return c
        jax.lax.fori_loop(0, 8, pro, 0)
        cp.wait()
        cpx.wait()

        ri = jax.lax.broadcasted_iota(jnp.int32, (L, L), 0)
        ci = jax.lax.broadcasted_iota(jnp.int32, (L, L), 1)
        mask = (ri < M) | (ri >= ci)

        def a_qkv(s, mem):
            r0 = pl.multiple_of(s * SEG, SEG)
            xs = xv[pl.ds(r0, SEG), :].astype(jnp.float32)
            h = jnp.concatenate([mem, xs], axis=0)
            w = pltpu.bitcast(wqkv[...], jnp.bfloat16)
            return _dot(h, w)
        def a_att(y):
            outs = []
            for i in range(H):
                q = y[:, i * 384:i * 384 + 128]
                k = y[:, i * 384 + 128:i * 384 + 256]
                v = y[:, i * 384 + 256:i * 384 + 384]
                sc = _dot(q, k, NT) * scale
                sc = jnp.where(mask, sc, -1e9)
                m = jnp.max(sc, axis=1, keepdims=True)
                e = jnp.exp(sc - m)
                p = e / jnp.sum(e, axis=1, keepdims=True)
                outs.append(_dot(p, v))
            return jnp.concatenate(outs, axis=1)
        def a_out(o, par):
            wo = pltpu.bitcast(wo32[...], jnp.bfloat16)
            y = _dot(o, wo)
            osta[par] = y[M:, :].astype(jnp.bfloat16)
            return y[:M, :]

        def slot_body(sg, mem):
            p = sg % 2
            jn = jnp.minimum(sg + 1, 7)
            @pl.when(sg < 7)
            def _():
                for cq in in_copies(sg + 1, 1 - p): cq.wait()
            q_copy(sg, p).wait()
            @pl.when(sg < 7)
            def _():
                q_copy(sg + 1, 1 - p).start()
            def step(i, mem):
                s = sg * 8 + i
                par = i % 2
                @pl.when(s >= 2)
                def _():
                    outa_copy(0, par).wait()
                    out_copy(0, 0, par * 2).wait(); out_copy(0, 0, par * 2 + 1).wait()
                if order == "A_first":
                    y = a_qkv(s, mem); o = a_att(y); mem = a_out(o, par)
                    if doB:
                        stage2(sg, p, i, par); stage1(jn, 1 - p, i)
                elif order == "B_first":
                    stage2(sg, p, i, par); stage1(jn, 1 - p, i)
                    y = a_qkv(s, mem); o = a_att(y); mem = a_out(o, par)
                elif order == "mid":
                    y = a_qkv(s, mem)
                    stage2(sg, p, i, par)
                    o = a_att(y)
                    stage1(jn, 1 - p, i)
                    mem = a_out(o, par)
                elif order == "mid2":
                    stage1(jn, 1 - p, i)
                    y = a_qkv(s, mem)
                    o = a_att(y)
                    stage2(sg, p, i, par)
                    mem = a_out(o, par)
                outa_copy(s, par).start()
                out_copy(sg, i, par * 2).start(); out_copy(sg, 15 - i, par * 2 + 1).start()
                return mem
            mem = jax.lax.fori_loop(0, 8, step, mem)
            @pl.when(sg < 6)
            def _():
                for cq in in_copies(sg + 2, p): cq.start()
            return mem
        mem = mem0_ref[...].astype(jnp.float32)
        jax.lax.fori_loop(0, 8, slot_body, mem)
        for par in range(2):
            outa_copy(0, par).wait()
            out_copy(0, 0, par * 2).wait(); out_copy(0, 0, par * 2 + 1).wait()

    def fn(x, mem0, wq, wk, wv, wo, q, k, v, shift_k, ssm_k, ssm_D):
        F, G = dft_consts()
        any_ = pl.BlockSpec(memory_space=pl.ANY)
        vm = pl.BlockSpec()
        wq2, wk2, wv2 = [w.reshape(DM * H, DH) for w in (wq, wk, wv)]
        out = pl.pallas_call(
            kern, out_shape=jax.ShapeDtypeStruct((S, 2 * D), jnp.bfloat16),
            in_specs=[any_, vm, any_, any_, any_, any_, any_, any_, any_, vm, any_, vm, vm, vm], out_specs=any_,
            scratch_shapes=[pltpu.VMEM((S, DM), jnp.bfloat16), pltpu.VMEM((DM * H // 2, DH), jnp.uint32),
                            pltpu.VMEM((DM // 2, H * 384), jnp.uint32), pltpu.VMEM((H * DH // 2, DM), jnp.uint32),
                            pltpu.VMEM((2, SEG, DM), jnp.bfloat16),
                            pltpu.SemaphoreType.DMA((2,)), pltpu.SemaphoreType.DMA((2,)),
                            pltpu.VMEM((2, S, 128), jnp.bfloat16), pltpu.VMEM((2, S, 128), jnp.bfloat16),
                            pltpu.VMEM((2, 128, S), jnp.bfloat16), pltpu.VMEM((2, S, 128), jnp.bfloat16),
                            pltpu.VMEM((S + 8, 128), jnp.float32), pltpu.VMEM((2, S, 128), jnp.float32),
                            pltpu.VMEM((2, 16, 256, 128), jnp.float32), pltpu.VMEM((2, 16, 256, 128), jnp.float32),
                            pltpu.VMEM((256, 128), jnp.float32), pltpu.VMEM((8, D), jnp.float32),
                            pltpu.VMEM((2, 256, 128), jnp.float32), pltpu.VMEM((4, 128, 128), jnp.bfloat16),
                            pltpu.SemaphoreType.DMA((2, 3)), pltpu.SemaphoreType.DMA((2,)), pltpu.SemaphoreType.DMA((4,))],
            compiler_params=pltpu.CompilerParams(vmem_limit_bytes=110 * 1024 * 1024),
        )(x.reshape(S, DM), mem0.reshape(M, DM), wq2, wk2, wv2, wo.reshape(H * DH, DM),
          q.reshape(S, D), k.reshape(S, D), v.reshape(S, D), shift_k, ssm_k, ssm_D.reshape(1, D),
          jnp.asarray(F, jnp.bfloat16), jnp.asarray(G, jnp.bfloat16))
        return out.reshape(1, S, 2 * D)
    return fn


@jax.jit
def pallas_concat_heads__memory_aug_recurrent_mem_tr__ssm_conv_h3__prompt_kernel(
    A_x, A_mem0, A_Wq, A_Wk, A_Wv, A_Wo, A_seg_len, B_q, B_k, B_v, B_shift_k, B_ssm_k, B_ssm_D,
):
    return make()(A_x, A_mem0, A_Wq, A_Wk, A_Wv, A_Wo, B_q, B_k, B_v, B_shift_k, B_ssm_k, B_ssm_D)
```

```python
import functools, itertools
import jax, jax.numpy as jnp, numpy as np
from jax.experimental import pallas as pl
from jax.experimental.pallas import tpu as pltpu

S, DM, H, DH, M, SEG = 2048, 1024, 32, 128, 8, 32
D = 1024
NSEG = S // SEG
L = M + SEG
P0 = 512
TS = 24
RING = 576
NT = (((1,), (1,)), ((), ()))
NN = (((1,), (0,)), ((), ()))
def _dot(a, b, dims=NN):
    return jax.lax.dot_general(a, b, dims, preferred_element_type=jnp.float32)

def dft_consts():
    N = 256; C = 128
    f_order = np.concatenate([np.arange(0, 128, 2), np.arange(1, 128, 2)])
    th = 2 * np.pi * np.outer(f_order + 0.5, np.arange(C)) / N
    F = np.concatenate([np.cos(th), -np.sin(th)], 0)
    G = np.concatenate([np.cos(th).T, -np.sin(th).T], 1) * (2.0 / N)
    return F.astype(np.float32), G.astype(np.float32)

def make(doB=True, G=4, lagS=1, lagP=2, OB=4, border="123", bpos=None, unroll=1, wo_split=0):
    scale = DH ** -0.5
    def kern(x_hbm, mem0_ref, wq_hbm, wk_hbm, wv_hbm, wo_hbm,
             q_hbm, k_hbm, v_hbm, sk_ref, w_hbm, dd_ref, f_ref, g_ref, out_hbm,
             xv, raw, wqkv, wo32, ring, osta, sems, osema,
             kin, vin, win, qin, kf32, kvb, uh, whp, yh, wprev, skt, ost, isem, qsem, osem):
        def in_copies(j, p):
            c = pl.multiple_of(j * 128, 128)
            return [pltpu.make_async_copy(k_hbm.at[:, pl.ds(c, 128)], kin.at[p], isem.at[p, 0]),
                    pltpu.make_async_copy(v_hbm.at[:, pl.ds(c, 128)], vin.at[p], isem.at[p, 1]),
                    pltpu.make_async_copy(w_hbm.at[pl.ds(c, 128), :], win.at[p], isem.at[p, 2])]
        def q_copy(j, p):
            c = pl.multiple_of(j * 128, 128)
            return pltpu.make_async_copy(q_hbm.at[:, pl.ds(c, 128)], qin.at[p], qsem.at[p])
        def out_copy(j, a, slot):
            return pltpu.make_async_copy(ost.at[slot], out_hbm.at[pl.ds(pl.multiple_of(a * 256, 256), 256), pl.ds(pl.multiple_of(D + j * 128, 128), 128)], osem.at[slot])
        def outa_copy(s, slot):
            return pltpu.make_async_copy(osta.at[slot], out_hbm.at[pl.ds(pl.multiple_of(s * SEG, SEG), SEG), pl.ds(0, DM)], osema.at[slot])

        for cp in in_copies(0, 0): cp.start()
        cpx = pltpu.make_async_copy(x_hbm, xv, sems.at[0]); cpx.start()
        skt[0:4, :] = sk_ref[...].astype(jnp.float32).T
        skt[4:5, :] = dd_ref[...].astype(jnp.float32)
        kf32[0:8, :] = jnp.zeros((8, 128), jnp.float32)
        F = f_ref[...]; G_ = g_ref[...]

        def stage1_gen(j, p, p3, i):
            r0 = pl.multiple_of(i * 256, 256)
            c0 = pl.multiple_of(j * 128, 128)
            taps = skt[:, pl.ds(c0, 128)]
            prev = jnp.where(i == 0, 0.0, wprev[...])
            for c in range(2):
                rc = pl.multiple_of(r0 + c * 128, 128)
                kf = kin[p, pl.ds(rc, 128), :].astype(jnp.float32)
                kf32[pl.ds(rc + 8, 128), :] = kf
                ks = (kf * taps[0:1] + kf32[pl.ds(rc + 7, 128), :] * taps[1:2]
                      + kf32[pl.ds(rc + 6, 128), :] * taps[2:3] + kf32[pl.ds(rc + 5, 128), :] * taps[3:4])
                kv = ks * vin[p, pl.ds(rc, 128), :].astype(jnp.float32)
                kvb[p3, pl.ds(rc, 128), :] = kv
                a = 2 * i + c
                uh[p, a] = _dot(F, kv)
                yield
                wt = win[p, :, pl.ds(pl.multiple_of(a * 128, 128), 128)]
                wh = _dot(F, wt, NT)
                pr, pi_ = prev[:128], prev[128:]
                re = jnp.concatenate([wh[0:64] - pi_[0:64], wh[64:128] + pi_[64:128]], 0)
                im = jnp.concatenate([wh[128:192] + pr[0:64], wh[192:256] - pr[64:128]], 0)
                whp[p, a, 0:128] = re
                whp[p, a, 128:256] = im
                prev = wh
                yield
            wprev[...] = prev

        def stage2_gen(p, i):
            for gg in range(2):
                rr = pl.multiple_of(i * 16 + gg * 8, 8)
                ri_ = pl.multiple_of(128 + i * 16 + gg * 8, 8)
                for b in range(16 // OB):
                    outs = list(range(b * OB, (b + 1) * OB))
                    accr = {}; acci = {}
                    W = {}
                    for ap in range(outs[-1] + 1):
                        ur = uh[p, ap, pl.ds(rr, 8), :]; ui = uh[p, ap, pl.ds(ri_, 8), :]
                        for a in outs:
                            m = a - ap
                            if m < 0: continue
                            if m not in W:
                                W[m] = (whp[p, m, pl.ds(rr, 8), :], whp[p, m, pl.ds(ri_, 8), :])
                            wr, wi = W[m]
                            tr = ur * wr - ui * wi; ti = ur * wi + ui * wr
                            accr[a] = tr if a not in accr else accr[a] + tr
                            acci[a] = ti if a not in acci else acci[a] + ti
                    for a in outs:
                        yh[p, a, pl.ds(rr, 8), :] = accr[a]
                        yh[p, a, pl.ds(ri_, 8), :] = acci[a]
                    yield

        def stage3_gen(j, p, p3, i, par):
            c0 = pl.multiple_of(j * 128, 128)
            dvec = skt[4:5, pl.ds(c0, 128)]
            for c in range(2):
                a = 2 * i + c
                y = _dot(G_, yh[p, a])
                r = pl.multiple_of(a * 128, 128)
                o = qin[p, pl.ds(r, 128), :].astype(jnp.float32) * (y + kvb[p3, pl.ds(r, 128), :] * dvec)
                ost[par, c * 128:(c + 1) * 128, :] = o.astype(jnp.bfloat16)
                yield

        for j, w_hbm_ in enumerate((wq_hbm, wk_hbm, wv_hbm)):
            cp = pltpu.make_async_copy(w_hbm_, raw.bitcast(jnp.bfloat16), sems.at[1])
            cp.start(); cp.wait()
            def per_hp(hp, c, j=j):
                for jj in range(8):
                    for t in range(8):
                        d0 = jj * 128 + t * 16
                        A = raw[pl.ds(d0 * 16 + hp, 8, stride=32), :]
                        B = raw[pl.ds(d0 * 16 + 16 + hp, 8, stride=32), :]
                        o0 = (A & jnp.uint32(0xFFFF)) | (B << 16)
                        o1 = (A >> 16) | (B & jnp.uint32(0xFFFF0000))
                        c0 = pl.multiple_of((2 * hp) * 384 + j * 128, 128)
                        c1 = pl.multiple_of((2 * hp + 1) * 384 + j * 128, 128)
                        wqkv[pl.ds(d0 // 2, 8), pl.ds(c0, 128)] = o0
                        wqkv[pl.ds(d0 // 2, 8), pl.ds(c1, 128)] = o1
                return c
            jax.lax.fori_loop(0, 16, per_hp, 0)
        cp = pltpu.make_async_copy(wo_hbm, wo32.bitcast(jnp.bfloat16), sems.at[1])
        cp.start()
        for cq in in_copies(1, 1): cq.start()
        q_copy(0, 0).start()
        for cq in in_copies(0, 0): cq.wait()
        def pro0(i, c):
            for _ in stage1_gen(0, 0, 0, i): pass
            return c
        jax.lax.fori_loop(0, 8, pro0, 0)
        for cq in in_copies(1, 1): cq.wait()
        for cq in in_copies(2, 0): cq.start()
        def pro1(i, c):
            for _ in stage1_gen(1, 1, 1, i): pass
            for _ in stage2_gen(0, i): pass
            return c
        jax.lax.fori_loop(0, 8, pro1, 0)
        cp.wait()
        cpx.wait()
        def proj(g, c):
            c0 = pl.multiple_of(g * 1536, 1536)
            w = pltpu.bitcast(wqkv[:, pl.ds(c0, 1536)], jnp.bfloat16)
            for rb in range(P0 // 256):
                ring[pl.ds(64 + rb * 256, 256), pl.ds(c0, 1536)] = _dot(xv[rb * 256:(rb + 1) * 256, :], w)
            return c
        jax.lax.fori_loop(0, 8, proj, 0)

        ri = jax.lax.broadcasted_iota(jnp.int32, (L, L), 0)
        ci = jax.lax.broadcasted_iota(jnp.int32, (L, L), 1)
        mask = (ri < M) | (ri >= ci)

        def slot_body(sg, mem):
            p = sg % 2
            p3 = jax.lax.rem(sg, 3); p3n = jax.lax.rem(sg + 2, 3)
            j1 = jnp.minimum(sg + 2, 7)
            @pl.when(sg < 6)
            def _():
                for cq in in_copies(sg + 2, p): cq.wait()
            q_copy(sg, p).wait()
            @pl.when(sg < 5)
            def _():
                for cq in in_copies(sg + 3, 1 - p): cq.start()
            @pl.when(sg < 7)
            def _():
                q_copy(sg + 1, 1 - p).start()
            def step(i, mem):
                s = sg * 8 + i
                par = i % 2
                @pl.when(s >= 2)
                def _():
                    outa_copy(0, par).wait()
                    out_copy(0, 0, par).wait()
                xr0 = pl.multiple_of(P0 + s * TS, 8)
                wr0 = pl.multiple_of(jax.lax.rem(s * TS, RING), 8)
                rr0 = pl.multiple_of(jax.lax.rem(s * SEG + 64, RING), 32)
                xs = xv[pl.ds(xr0, TS), :].astype(jnp.float32)
                h = jnp.concatenate([mem, xs], axis=0).astype(jnp.bfloat16)
                NG = H // G
                if doB:
                    gens = {"1": lambda: stage1_gen(j1, p, p3n, i), "2": lambda: stage2_gen(1 - p, i),
                            "3": lambda: stage3_gen(sg, p, p3, i, par)}
                    bgen = itertools.chain(*[gens[c]() for c in border])
                else:
                    bgen = iter(())
                nb = 4 + 2 * (16 // OB) + 2
                ys = {}; ps = {}; outs = []
                for t in range(NG + lagP):
                    if t < NG:
                        w = pltpu.bitcast(wqkv[:, t * G * 384:(t + 1) * G * 384], jnp.bfloat16)
                        ys[t] = _dot(h, w)
                    if 0 <= t - lagS < NG:
                        tt = t - lagS
                        y = ys[tt]; pl_ = []
                        ring[pl.ds(wr0, TS), tt * G * 384:(tt + 1) * G * 384] = y[M:, :]
                        for ii in range(G):
                            c = (tt * G + ii) * 384
                            q = jnp.concatenate([y[:M, ii * 384:ii * 384 + 128], ring[pl.ds(rr0, SEG), c:c + 128]], 0)
                            k = jnp.concatenate([y[:M, ii * 384 + 128:ii * 384 + 256], ring[pl.ds(rr0, SEG), c + 128:c + 256]], 0)
                            sc = _dot(q, k, NT) * scale
                            sc = jnp.where(mask, sc, -1e9)
                            m = jnp.max(sc, axis=1, keepdims=True)
                            e = jnp.exp(sc - m)
                            pl_.append(e / jnp.sum(e, axis=1, keepdims=True))
                        ps[tt] = pl_
                    if 0 <= t - lagP < NG:
                        tt = t - lagP
                        y = ys[tt]
                        for ii in range(G):
                            c = (tt * G + ii) * 384
                            v = jnp.concatenate([y[:M, ii * 384 + 256:ii * 384 + 384], ring[pl.ds(rr0, SEG), c + 256:c + 384]], 0)
                            outs.append(_dot(ps[tt][ii], v))
                    if t < NG:
                        if bpos is None:
                            tgt = (t + 1) * nb // NG - t * nb // NG
                        else:
                            tgt = bpos[t]
                        for _ in range(tgt):
                            next(bgen, None)
                wo = pltpu.bitcast(wo32[...], jnp.bfloat16)
                if wo_split:
                    c = wo_split * 128
                    y = _dot(jnp.concatenate(outs[:wo_split], axis=1), wo[:c])
                    for _ in bgen: pass
                    y = y + _dot(jnp.concatenate(outs[wo_split:], axis=1), wo[c:])
                else:
                    for _ in bgen: pass
                    o = jnp.concatenate(outs, axis=1)
                    y = _dot(o, wo)
                osta[par] = y[M:, :].astype(jnp.bfloat16)
                mem = y[:M, :]
                outa_copy(s, par).start()
                out_copy(sg, i, par).start()
                return mem
            mem = jax.lax.fori_loop(0, 8, step, mem, unroll=unroll)
            return mem
        mem = mem0_ref[...].astype(jnp.float32)
        jax.lax.fori_loop(0, 8, slot_body, mem)
        for par in range(2):
            outa_copy(0, par).wait()
            out_copy(0, 0, par).wait()

    def fn(x, mem0, wq, wk, wv, wo, q, k, v, shift_k, ssm_k, ssm_D):
        F, G = dft_consts()
        any_ = pl.BlockSpec(memory_space=pl.ANY)
        vm = pl.BlockSpec()
        wq2, wk2, wv2 = [w.reshape(DM * H, DH) for w in (wq, wk, wv)]
        out = pl.pallas_call(
            kern, out_shape=jax.ShapeDtypeStruct((S, 2 * D), jnp.bfloat16),
            in_specs=[any_, vm, any_, any_, any_, any_, any_, any_, any_, vm, any_, vm, vm, vm], out_specs=any_,
            scratch_shapes=[pltpu.VMEM((S, DM), jnp.bfloat16), pltpu.VMEM((DM * H // 2, DH), jnp.uint32),
                            pltpu.VMEM((DM // 2, H * 384), jnp.uint32), pltpu.VMEM((H * DH // 2, DM), jnp.uint32),
                            pltpu.VMEM((RING, H * 384), jnp.float32),
                            pltpu.VMEM((2, SEG, DM), jnp.bfloat16),
                            pltpu.SemaphoreType.DMA((2,)), pltpu.SemaphoreType.DMA((2,)),
                            pltpu.VMEM((2, S, 128), jnp.bfloat16), pltpu.VMEM((2, S, 128), jnp.bfloat16),
                            pltpu.VMEM((2, 128, S), jnp.bfloat16), pltpu.VMEM((2, S, 128), jnp.bfloat16),
                            pltpu.VMEM((S + 8, 128), jnp.float32), pltpu.VMEM((3, S, 128), jnp.float32),
                            pltpu.VMEM((2, 16, 256, 128), jnp.float32), pltpu.VMEM((2, 16, 256, 128), jnp.float32),
                            pltpu.VMEM((2, 16, 256, 128), jnp.float32),
                            pltpu.VMEM((256, 128), jnp.float32), pltpu.VMEM((8, D), jnp.float32),
                            pltpu.VMEM((2, 256, 128), jnp.bfloat16),
                            pltpu.SemaphoreType.DMA((2, 3)), pltpu.SemaphoreType.DMA((2,)), pltpu.SemaphoreType.DMA((2,))],
            compiler_params=pltpu.CompilerParams(vmem_limit_bytes=120 * 1024 * 1024),
        )(x.reshape(S, DM), mem0.reshape(M, DM), wq2, wk2, wv2, wo.reshape(H * DH, DM),
          q.reshape(S, D), k.reshape(S, D), v.reshape(S, D), shift_k, ssm_k, ssm_D.reshape(1, D),
          jnp.asarray(F, jnp.bfloat16), jnp.asarray(G, jnp.bfloat16))
        return out.reshape(1, S, 2 * D)
    return fn


@jax.jit
def pallas_concat_heads__memory_aug_recurrent_mem_tr__ssm_conv_h3__prompt_kernel(
    A_x, A_mem0, A_Wq, A_Wk, A_Wv, A_Wo, A_seg_len, B_q, B_k, B_v, B_shift_k, B_ssm_k, B_ssm_D,
):
    return make()(A_x, A_mem0, A_Wq, A_Wk, A_Wv, A_Wo, B_q, B_k, B_v, B_shift_k, B_ssm_k, B_ssm_D)
```

```python
import functools, itertools
import jax, jax.numpy as jnp, numpy as np
from jax.experimental import pallas as pl
from jax.experimental.pallas import tpu as pltpu

S, DM, H, DH, M, SEG = 2048, 1024, 32, 128, 8, 32
D = 1024
NSEG = S // SEG
L = M + SEG
P0 = 512
TS = 24
RING = 576
NT = (((1,), (1,)), ((), ()))
NN = (((1,), (0,)), ((), ()))
def _dot(a, b, dims=NN):
    return jax.lax.dot_general(a, b, dims, preferred_element_type=jnp.float32)

def dft_consts():
    N = 256; C = 128
    f_order = np.concatenate([np.arange(0, 128, 2), np.arange(1, 128, 2)])
    th = 2 * np.pi * np.outer(f_order + 0.5, np.arange(C)) / N
    F = np.concatenate([np.cos(th), -np.sin(th)], 0)
    G = np.concatenate([np.cos(th).T, -np.sin(th).T], 1) * (2.0 / N)
    return F.astype(np.float32), G.astype(np.float32)

def make(doB=True, G=4, lagS=1, lagP=2, OB=4, border="123", bpos=None, unroll=1, wo_split=0):
    scale = DH ** -0.5
    def kern(x_hbm, mem0_ref, wq_hbm, wk_hbm, wv_hbm, wo_hbm,
             q_hbm, k_hbm, v_hbm, sk_ref, w_hbm, dd_ref, f_ref, g_ref, out_hbm,
             xv, wqkv, wo32, ring, osta, sems, osema, wsem, xsem,
             kin, vin, win, qin, kf32, kvb, uh, whp, yh, wprev, skt, ost, isem, qsem, osem):
        def in_copies(j, p):
            c = pl.multiple_of(j * 128, 128)
            return [pltpu.make_async_copy(k_hbm.at[:, pl.ds(c, 128)], kin.at[p], isem.at[p, 0]),
                    pltpu.make_async_copy(v_hbm.at[:, pl.ds(c, 128)], vin.at[p], isem.at[p, 1]),
                    pltpu.make_async_copy(w_hbm.at[pl.ds(c, 128), :], win.at[p], isem.at[p, 2])]
        def q_copy(j, p):
            c = pl.multiple_of(j * 128, 128)
            return pltpu.make_async_copy(q_hbm.at[:, pl.ds(c, 128)], qin.at[p], qsem.at[p])
        def out_copy(j, a, slot):
            return pltpu.make_async_copy(ost.at[slot], out_hbm.at[pl.ds(pl.multiple_of(a * 256, 256), 256), pl.ds(pl.multiple_of(D + j * 128, 128), 128)], osem.at[slot])
        def outa_copy(s, slot):
            return pltpu.make_async_copy(osta.at[slot], out_hbm.at[pl.ds(pl.multiple_of(s * SEG, SEG), SEG), pl.ds(0, DM)], osema.at[slot])

        wsrc = [w.bitcast(jnp.uint32) for w in (wq_hbm, wk_hbm, wv_hbm)]
        def w_copies(hp):
            out = []
            for j in range(3):
                for par in range(2):
                    col = pl.multiple_of((2 * hp + par) * 384 + j * 128, 128)
                    out.append(pltpu.make_async_copy(wsrc[j].at[:, par, hp, :], wqkv.at[:, pl.ds(col, 128)], wsem.at[hp % 4]))
            return out
        def w_inter(hp):
            for j in range(3):
                c0 = pl.multiple_of((2 * hp) * 384 + j * 128, 128); c1 = pl.multiple_of((2 * hp + 1) * 384 + j * 128, 128)
                A = wqkv[:, pl.ds(c0, 128)]; B = wqkv[:, pl.ds(c1, 128)]
                wqkv[:, pl.ds(c0, 128)] = (A & jnp.uint32(0xFFFF)) | (B << 16)
                wqkv[:, pl.ds(c1, 128)] = (A >> 16) | (B & jnp.uint32(0xFFFF0000))
        def wo_copy(part):
            r = pl.multiple_of(part * 512, 512)
            return pltpu.make_async_copy(wo_hbm.at[pl.ds(r, 512), :], wo32.bitcast(jnp.bfloat16).at[pl.ds(r, 512), :], sems.at[1])
        def x_copy(part):
            r = pl.multiple_of(part * 512, 512)
            return pltpu.make_async_copy(x_hbm.at[pl.ds(r, 512), :], xv.at[pl.ds(r, 512), :], sems.at[0] if False else xsem.at[part])
        x_copy(0).start()
        for cq in w_copies(0): cq.start()
        for cq in w_copies(1): cq.start()
        for cq in in_copies(0, 0): cq.start()
        skt[0:4, :] = sk_ref[...].astype(jnp.float32).T
        skt[4:5, :] = dd_ref[...].astype(jnp.float32)
        kf32[0:8, :] = jnp.zeros((8, 128), jnp.float32)
        F = f_ref[...]; G_ = g_ref[...]

        def stage1_gen(j, p, p3, i):
            r0 = pl.multiple_of(i * 256, 256)
            c0 = pl.multiple_of(j * 128, 128)
            taps = skt[:, pl.ds(c0, 128)]
            prev = jnp.where(i == 0, 0.0, wprev[...])
            for c in range(2):
                rc = pl.multiple_of(r0 + c * 128, 128)
                kf = kin[p, pl.ds(rc, 128), :].astype(jnp.float32)
                kf32[pl.ds(rc + 8, 128), :] = kf
                ks = (kf * taps[0:1] + kf32[pl.ds(rc + 7, 128), :] * taps[1:2]
                      + kf32[pl.ds(rc + 6, 128), :] * taps[2:3] + kf32[pl.ds(rc + 5, 128), :] * taps[3:4])
                kv = ks * vin[p, pl.ds(rc, 128), :].astype(jnp.float32)
                kvb[p3, pl.ds(rc, 128), :] = kv
                a = 2 * i + c
                uh[p, a] = _dot(F, kv)
                yield
                wt = win[p, :, pl.ds(pl.multiple_of(a * 128, 128), 128)]
                wh = _dot(F, wt, NT)
                pr, pi_ = prev[:128], prev[128:]
                re = jnp.concatenate([wh[0:64] - pi_[0:64], wh[64:128] + pi_[64:128]], 0)
                im = jnp.concatenate([wh[128:192] + pr[0:64], wh[192:256] - pr[64:128]], 0)
                whp[p, a, 0:128] = re
                whp[p, a, 128:256] = im
                prev = wh
                yield
            wprev[...] = prev

        def stage2_gen(p, i):
            for gg in range(2):
                rr = pl.multiple_of(i * 16 + gg * 8, 8)
                ri_ = pl.multiple_of(128 + i * 16 + gg * 8, 8)
                for b in range(16 // OB):
                    outs = list(range(b * OB, (b + 1) * OB))
                    accr = {}; acci = {}
                    W = {}
                    for ap in range(outs[-1] + 1):
                        ur = uh[p, ap, pl.ds(rr, 8), :]; ui = uh[p, ap, pl.ds(ri_, 8), :]
                        for a in outs:
                            m = a - ap
                            if m < 0: continue
                            if m not in W:
                                W[m] = (whp[p, m, pl.ds(rr, 8), :], whp[p, m, pl.ds(ri_, 8), :])
                            wr, wi = W[m]
                            tr = ur * wr - ui * wi; ti = ur * wi + ui * wr
                            accr[a] = tr if a not in accr else accr[a] + tr
                            acci[a] = ti if a not in acci else acci[a] + ti
                    for a in outs:
                        yh[p, a, pl.ds(rr, 8), :] = accr[a]
                        yh[p, a, pl.ds(ri_, 8), :] = acci[a]
                    yield

        def stage3_gen(j, p, p3, i, par):
            c0 = pl.multiple_of(j * 128, 128)
            dvec = skt[4:5, pl.ds(c0, 128)]
            for c in range(2):
                a = 2 * i + c
                y = _dot(G_, yh[p, a])
                r = pl.multiple_of(a * 128, 128)
                o = qin[p, pl.ds(r, 128), :].astype(jnp.float32) * (y + kvb[p3, pl.ds(r, 128), :] * dvec)
                ost[par, c * 128:(c + 1) * 128, :] = o.astype(jnp.bfloat16)
                yield

        def proj_half(hp, rb):
            c0 = pl.multiple_of(hp * 768, 768)
            w = pltpu.bitcast(wqkv[:, pl.ds(c0, 768)], jnp.bfloat16)
            ring[pl.ds(64 + rb * 256, 256), pl.ds(c0, 768)] = _dot(xv[rb * 256:(rb + 1) * 256, :], w)
        def b_unit(u, kind):
            if kind == 0:
                for _ in stage1_gen(0, 0, 0, u): pass
            else:
                for _ in stage1_gen(1, 1, 1, u): pass
                for _ in stage2_gen(0, u): pass
        def startup_iter(it, kind, last=False):
            if not last:
                @pl.when(it < 14)
                def _():
                    for cq in w_copies(it + 2): cq.start()
            if kind == -1:
                for cq in in_copies(1, 1): cq.start()
            elif kind == 0:
                @pl.when(it == 1)
                def _():
                    q_copy(0, 0).start()
                @pl.when(it >= 2)
                def _():
                    wo_copy(it - 2).start()
            elif kind == 1:
                @pl.when(it == 9)
                def _():
                    wo_copy(7).start()
                @pl.when((it >= 10) & (it < 13))
                def _():
                    x_copy(it - 9).start()
                @pl.when(it == 13)
                def _():
                    for cq in in_copies(2, 0): cq.start()
            proj_half(it, 0)
            if not last:
                for cq in w_copies(it + 1): cq.wait()
                w_inter(it + 1)
            if kind == 0:
                b_unit(it - 1, 0)
            elif kind == 1:
                b_unit(it - 9, 1)
            elif kind == 2:
                b_unit(6, 1); b_unit(7, 1)
            proj_half(it, 1)
        x_copy(0).wait()
        for cq in w_copies(0): cq.wait()
        w_inter(0)
        startup_iter(0, -1)
        for cq in in_copies(0, 0): cq.wait()
        def loop_a(it, c):
            startup_iter(it, 0); return c
        jax.lax.fori_loop(1, 9, loop_a, 0)
        for cq in in_copies(1, 1): cq.wait()
        def loop_b(it, c):
            startup_iter(it, 1); return c
        jax.lax.fori_loop(9, 15, loop_b, 0)
        startup_iter(15, 2, last=True)
        for part in range(8): wo_copy(part).wait()
        for part in range(1, 4): x_copy(part).wait()

        ri = jax.lax.broadcasted_iota(jnp.int32, (L, L), 0)
        ci = jax.lax.broadcasted_iota(jnp.int32, (L, L), 1)
        mask = (ri < M) | (ri >= ci)

        def slot_body(sg, mem):
            p = sg % 2
            p3 = jax.lax.rem(sg, 3); p3n = jax.lax.rem(sg + 2, 3)
            j1 = jnp.minimum(sg + 2, 7)
            @pl.when(sg < 6)
            def _():
                for cq in in_copies(sg + 2, p): cq.wait()
            q_copy(sg, p).wait()
            @pl.when(sg < 5)
            def _():
                for cq in in_copies(sg + 3, 1 - p): cq.start()
            @pl.when(sg < 7)
            def _():
                q_copy(sg + 1, 1 - p).start()
            def step(i, mem):
                s = sg * 8 + i
                par = i % 2
                @pl.when(s >= 2)
                def _():
                    outa_copy(0, par).wait()
                    out_copy(0, 0, par).wait()
                xr0 = pl.multiple_of(P0 + s * TS, 8)
                wr0 = pl.multiple_of(jax.lax.rem(s * TS, RING), 8)
                rr0 = pl.multiple_of(jax.lax.rem(s * SEG + 64, RING), 32)
                xs = xv[pl.ds(xr0, TS), :].astype(jnp.float32)
                h = jnp.concatenate([mem, xs], axis=0).astype(jnp.bfloat16)
                NG = H // G
                if doB:
                    gens = {"1": lambda: stage1_gen(j1, p, p3n, i), "2": lambda: stage2_gen(1 - p, i),
                            "3": lambda: stage3_gen(sg, p, p3, i, par)}
                    bgen = itertools.chain(*[gens[c]() for c in border])
                else:
                    bgen = iter(())
                nb = 4 + 2 * (16 // OB) + 2
                ys = {}; ps = {}; outs = []
                for t in range(NG + lagP):
                    if t < NG:
                        w = pltpu.bitcast(wqkv[:, t * G * 384:(t + 1) * G * 384], jnp.bfloat16)
                        ys[t] = _dot(h, w)
                    if 0 <= t - lagS < NG:
                        tt = t - lagS
                        y = ys[tt]; pl_ = []
                        ring[pl.ds(wr0, TS), tt * G * 384:(tt + 1) * G * 384] = y[M:, :]
                        for ii in range(G):
                            c = (tt * G + ii) * 384
                            q = jnp.concatenate([y[:M, ii * 384:ii * 384 + 128], ring[pl.ds(rr0, SEG), c:c + 128]], 0)
                            k = jnp.concatenate([y[:M, ii * 384 + 128:ii * 384 + 256], ring[pl.ds(rr0, SEG), c + 128:c + 256]], 0)
                            sc = _dot(q, k, NT) * scale
                            sc = jnp.where(mask, sc, -1e9)
                            m = jnp.max(sc, axis=1, keepdims=True)
                            e = jnp.exp(sc - m)
                            pl_.append(e / jnp.sum(e, axis=1, keepdims=True))
                        ps[tt] = pl_
                    if 0 <= t - lagP < NG:
                        tt = t - lagP
                        y = ys[tt]
                        for ii in range(G):
                            c = (tt * G + ii) * 384
                            v = jnp.concatenate([y[:M, ii * 384 + 256:ii * 384 + 384], ring[pl.ds(rr0, SEG), c + 256:c + 384]], 0)
                            outs.append(_dot(ps[tt][ii], v))
                    if t < NG:
                        if bpos is None:
                            tgt = (t + 1) * nb // NG - t * nb // NG
                        else:
                            tgt = bpos[t]
                        for _ in range(tgt):
                            next(bgen, None)
                wo = pltpu.bitcast(wo32[...], jnp.bfloat16)
                if wo_split:
                    c = wo_split * 128
                    y = _dot(jnp.concatenate(outs[:wo_split], axis=1), wo[:c])
                    for _ in bgen: pass
                    y = y + _dot(jnp.concatenate(outs[wo_split:], axis=1), wo[c:])
                else:
                    for _ in bgen: pass
                    o = jnp.concatenate(outs, axis=1)
                    y = _dot(o, wo)
                osta[par] = y[M:, :].astype(jnp.bfloat16)
                mem = y[:M, :]
                outa_copy(s, par).start()
                out_copy(sg, i, par).start()
                return mem
            mem = jax.lax.fori_loop(0, 8, step, mem, unroll=unroll)
            return mem
        mem = mem0_ref[...].astype(jnp.float32)
        jax.lax.fori_loop(0, 8, slot_body, mem)
        for par in range(2):
            outa_copy(0, par).wait()
            out_copy(0, 0, par).wait()

    def fn(x, mem0, wq, wk, wv, wo, q, k, v, shift_k, ssm_k, ssm_D):
        F, G = dft_consts()
        any_ = pl.BlockSpec(memory_space=pl.ANY)
        vm = pl.BlockSpec()
        wq2, wk2, wv2 = [w.reshape(DM // 2, 2, H, DH) for w in (wq, wk, wv)]
        out = pl.pallas_call(
            kern, out_shape=jax.ShapeDtypeStruct((S, 2 * D), jnp.bfloat16),
            in_specs=[any_, vm, any_, any_, any_, any_, any_, any_, any_, vm, any_, vm, vm, vm], out_specs=any_,
            scratch_shapes=[pltpu.VMEM((S, DM), jnp.bfloat16),
                            pltpu.VMEM((DM // 2, H * 384), jnp.uint32), pltpu.VMEM((H * DH // 2, DM), jnp.uint32),
                            pltpu.VMEM((RING, H * 384), jnp.float32),
                            pltpu.VMEM((2, SEG, DM), jnp.bfloat16),
                            pltpu.SemaphoreType.DMA((2,)), pltpu.SemaphoreType.DMA((2,)), pltpu.SemaphoreType.DMA((4,)), pltpu.SemaphoreType.DMA((4,)),
                            pltpu.VMEM((2, S, 128), jnp.bfloat16), pltpu.VMEM((2, S, 128), jnp.bfloat16),
                            pltpu.VMEM((2, 128, S), jnp.bfloat16), pltpu.VMEM((2, S, 128), jnp.bfloat16),
                            pltpu.VMEM((S + 8, 128), jnp.float32), pltpu.VMEM((3, S, 128), jnp.float32),
                            pltpu.VMEM((2, 16, 256, 128), jnp.float32), pltpu.VMEM((2, 16, 256, 128), jnp.float32),
                            pltpu.VMEM((2, 16, 256, 128), jnp.float32),
                            pltpu.VMEM((256, 128), jnp.float32), pltpu.VMEM((8, D), jnp.float32),
                            pltpu.VMEM((2, 256, 128), jnp.bfloat16),
                            pltpu.SemaphoreType.DMA((2, 3)), pltpu.SemaphoreType.DMA((2,)), pltpu.SemaphoreType.DMA((2,))],
            compiler_params=pltpu.CompilerParams(vmem_limit_bytes=120 * 1024 * 1024),
        )(x.reshape(S, DM), mem0.reshape(M, DM), wq2, wk2, wv2, wo.reshape(H * DH, DM),
          q.reshape(S, D), k.reshape(S, D), v.reshape(S, D), shift_k, ssm_k, ssm_D.reshape(1, D),
          jnp.asarray(F, jnp.bfloat16), jnp.asarray(G, jnp.bfloat16))
        return out.reshape(1, S, 2 * D)
    return fn


@jax.jit
def pallas_concat_heads__memory_aug_recurrent_mem_tr__ssm_conv_h3__prompt_kernel(
    A_x, A_mem0, A_Wq, A_Wk, A_Wv, A_Wo, A_seg_len, B_q, B_k, B_v, B_shift_k, B_ssm_k, B_ssm_D,
):
    return make()(A_x, A_mem0, A_Wq, A_Wk, A_Wv, A_Wo, B_q, B_k, B_v, B_shift_k, B_ssm_k, B_ssm_D)
```

```python
import functools
import jax, jax.numpy as jnp, numpy as np
from jax.experimental import pallas as pl
from jax.experimental.pallas import tpu as pltpu

S, DM, H, DH, M, SEG = 2048, 1024, 32, 128, 8, 32
D = 1024
NSEG = S // SEG
L = M + SEG
P0 = 512
TS = 24
RING = 576
NT = (((1,), (1,)), ((), ()))
NN = (((1,), (0,)), ((), ()))
def _dot(a, b, dims=NN):
    return jax.lax.dot_general(a, b, dims, preferred_element_type=jnp.float32)

def dft_consts():
    N = 256; C = 128
    f_order = np.concatenate([np.arange(0, 128, 2), np.arange(1, 128, 2)])
    th = 2 * np.pi * np.outer(f_order + 0.5, np.arange(C)) / N
    F = np.concatenate([np.cos(th), -np.sin(th)], 0)
    G = np.concatenate([np.cos(th).T, -np.sin(th).T], 1) * (2.0 / N)
    return F.astype(np.float32), G.astype(np.float32)

def plan_default(NG):
    pre = {0:['b1','b1'],1:['b1','b1'],2:['b2','b2'],3:['b2','b2'],4:['b2','b2'],5:['b2','b2'],8:['b3','b3']}
    P = []
    for t in range(NG + 3):
        if t < NG: P.append(("mm", t))
        if 0 <= t - 1 < NG: P += [("st", t - 1), ("qk", t - 1)]
        if 0 <= t - 3 < NG: P.append(("pv", t - 3))
        P += [(b, 1) for b in pre.get(t, [])]
    P.append(("wo", (0, NG)))
    return P

def make(G=4, OB=4, plan=None, unroll=4, smx=1, noatt=0, staged=True, ua=1, ub=1, scopes=None, slotdma=True, NSL=8, doB=True, PM=256, bsel=('b1','b2','b3'),
         splanA=(("p", 9), ("b1", 9))):
    if plan is None:
        plan = plan_default
    scale = DH ** -0.5
    LOG2E = float(np.log2(np.e))
    NG = H // G

    def kern(x_hbm, mem0_hbm, wq_hbm, wk_hbm, wv_hbm, wo_hbm,
             q_hbm, k_hbm, v_hbm, sk_hbm, w_hbm, dd_hbm, f_hbm, g_hbm, out_hbm,
             xv, raw, wqkv, wo32, ring, osta, mem0v, skv, ddv, fv, gv,
             kin, vin, win, qin, kf32, uh, whp, yh, wprev, skt, ost, dummy_a, dummy_b, ostaS, ostS, dummyS,
             wsem, xsem, wosem, smsem, osema, isem, qsem, osem):
        def in_copies(j, p):
            c = pl.multiple_of(j * 128, 128)
            return [pltpu.make_async_copy(k_hbm.at[:, pl.ds(c, 128)], kin.at[p], isem.at[p, 0]),
                    pltpu.make_async_copy(v_hbm.at[:, pl.ds(c, 128)], vin.at[p], isem.at[p, 1]),
                    pltpu.make_async_copy(w_hbm.at[pl.ds(c, 128), :], win.at[p], isem.at[p, 2])]
        def q_copy(j, p):
            c = pl.multiple_of(j * 128, 128)
            return pltpu.make_async_copy(q_hbm.at[:, pl.ds(c, 128)], qin.at[p], qsem.at[p])
        def out_copy(j, i, slot):
            return pltpu.make_async_copy(ost.at[slot], out_hbm.at[pl.ds(pl.multiple_of(i * 256, 256), 256), pl.ds(pl.multiple_of(D + j * 128, 128), 128)], osem.at[slot])
        def outa_slot_copy(sg, slot):
            return pltpu.make_async_copy(ostaS.at[slot], out_hbm.at[pl.ds(pl.multiple_of(sg * 256, 256), 256), pl.ds(0, DM)], osema.at[slot])
        def outb_slot_copy(j, slot):
            return pltpu.make_async_copy(ostS.at[slot], out_hbm.at[:, pl.ds(pl.multiple_of(D + j * 128, 128), 128)], osem.at[slot])
        def outa_copy(s, slot):
            return pltpu.make_async_copy(osta.at[slot], out_hbm.at[pl.ds(pl.multiple_of(s * SEG, SEG), SEG), pl.ds(0, DM)], osema.at[slot])
        wsrc = [w.bitcast(jnp.uint32) for w in (wq_hbm, wk_hbm, wv_hbm)]
        def w_copies(hp):
            slot = hp % 3
            return [pltpu.make_async_copy(wsrc[j].at[:, par, hp, :], raw.at[slot, 2 * j + par], wsem.at[slot])
                    for j in range(3) for par in range(2)]
        def wo_copy(part):
            r = pl.multiple_of(part * 512, 512)
            return pltpu.make_async_copy(wo_hbm.at[pl.ds(r, 512), :], wo32.bitcast(jnp.bfloat16).at[pl.ds(r, 512), :], wosem)
        def x_copy(part):
            r = pl.multiple_of(part * 512, 512)
            return pltpu.make_async_copy(x_hbm.at[pl.ds(r, 512), :], xv.at[pl.ds(r, 512), :], xsem.at[part])
        small = [pltpu.make_async_copy(a, b, smsem.at[n]) for n, (a, b) in enumerate(
            ((mem0_hbm, mem0v), (sk_hbm, skv), (dd_hbm, ddv), (f_hbm, fv), (g_hbm, gv)))]

        x_copy(0).start()
        for cq in w_copies(0): cq.start()
        for cq in small: cq.start()
        if not staged:
            for cq in w_copies(1): cq.start()
            for cq in in_copies(0, 0): cq.start()
        kf32[0:8, :] = jnp.zeros((8, 128), jnp.float32)
        yh[1] = jnp.zeros((16, 256, 128), jnp.float32)
        qin[1] = jnp.zeros((S, 128), jnp.bfloat16)
        wprev[...] = jnp.zeros((256, 128), jnp.float32)
        for par in range(2):
            osta[par] = jnp.zeros((SEG, DM), jnp.bfloat16)
            ost[par] = jnp.zeros((256, 128), jnp.bfloat16)
        if not slotdma:
            for par in range(2):
                pltpu.make_async_copy(osta.at[par], dummy_a.at[par], osema.at[par]).start()
                pltpu.make_async_copy(ost.at[par], dummy_b.at[par], osem.at[par]).start()
        for cq in small: cq.wait()
        skt[0:4, :] = skv[...].astype(jnp.float32)
        skt[4:5, :] = ddv[...].astype(jnp.float32).reshape(1, D)
        skt[5:8, :] = jnp.zeros((3, D), jnp.float32)

        def stage1_gen(j, p, i):
            r0 = pl.multiple_of(i * 256, 256)
            c0 = pl.multiple_of(j * 128, 128)
            taps = skt[:, pl.ds(c0, 128)]
            first = i == 0
            prev = jnp.where(first, 0.0, wprev[...])
            for c in range(2):
                rc = pl.multiple_of(r0 + c * 128, 128)
                kf = kin[p, pl.ds(rc, 128), :].astype(jnp.float32)
                kf32[pl.ds(rc + 8, 128), :] = kf
                ks = (kf * taps[0:1] + kf32[pl.ds(rc + 7, 128), :] * taps[1:2]
                      + kf32[pl.ds(rc + 6, 128), :] * taps[2:3] + kf32[pl.ds(rc + 5, 128), :] * taps[3:4])
                kv = ks * vin[p, pl.ds(rc, 128), :].astype(jnp.float32)
                a = 2 * i + c
                uh[p, a] = _dot(fv[...], kv)
                yield
                wt = win[p, :, pl.ds(pl.multiple_of(a * 128, 128), 128)]
                wh = _dot(fv[...], wt, NT)
                pr, pi_ = prev[:128], prev[128:]
                re = jnp.concatenate([wh[0:64] - pi_[0:64], wh[64:128] + pi_[64:128]], 0)
                im = jnp.concatenate([wh[128:192] + pr[0:64], wh[192:256] - pr[64:128]], 0)
                if c == 0:
                    re = re + jnp.where(first, taps[4:5], 0.0)
                whp[p, a, 0:128] = re
                whp[p, a, 128:256] = im
                prev = wh
                yield
            wprev[...] = prev

        def stage2_gen(p, i):
            for gg in range(2):
                rr = pl.multiple_of(i * 16 + gg * 8, 8)
                ri_ = pl.multiple_of(128 + i * 16 + gg * 8, 8)
                for b in range(16 // OB):
                    outs = list(range(b * OB, (b + 1) * OB))
                    accr = {}; acci = {}; W = {}
                    for ap in range(outs[-1] + 1):
                        ur = uh[p, ap, pl.ds(rr, 8), :]; ui = uh[p, ap, pl.ds(ri_, 8), :]
                        for a in outs:
                            m = a - ap
                            if m < 0: continue
                            if m not in W:
                                W[m] = (whp[p, m, pl.ds(rr, 8), :], whp[p, m, pl.ds(ri_, 8), :])
                            wr, wi = W[m]
                            tr = ur * wr - ui * wi; ti = ur * wi + ui * wr
                            accr[a] = tr if a not in accr else accr[a] + tr
                            acci[a] = ti if a not in acci else acci[a] + ti
                    for a in outs:
                        yh[p, a, pl.ds(rr, 8), :] = accr[a]
                        yh[p, a, pl.ds(ri_, 8), :] = acci[a]
                    yield

        def stage3_gen(p, i, par):
            for c in range(2):
                a = 2 * i + c
                y = _dot(gv[...], yh[p, a])
                r = pl.multiple_of(a * 128, 128)
                o = qin[p, pl.ds(r, 128), :].astype(jnp.float32) * y
                if slotdma:
                    ostS[p, pl.ds(r, 128), :] = o.astype(jnp.bfloat16)
                else:
                    ost[par, c * 128:(c + 1) * 128, :] = o.astype(jnp.bfloat16)
                yield

        def proj_gen(hp):
            slot = hp % 3
            lo = []; hi = []
            for j in range(3):
                A = raw[slot, 2 * j]; B = raw[slot, 2 * j + 1]
                lo.append((A & jnp.uint32(0xFFFF)) | (B << 16))
                hi.append((A >> 16) | (B & jnp.uint32(0xFFFF0000)))
            w32 = jnp.concatenate(lo + hi, axis=1)
            c0 = pl.multiple_of(hp * 768, 768)
            wqkv[:, pl.ds(c0, 768)] = w32
            w = pltpu.bitcast(w32, jnp.bfloat16)
            for rb in range(P0 // PM):
                ring[pl.ds(64 + rb * PM, PM), pl.ds(c0, 768)] = _dot(xv[rb * PM:(rb + 1) * PM, :], w)
                yield
        def run_plan(pl0, gens):
            for op, n in pl0:
                if op in gens:
                    for _ in range(n): next(gens[op], None)
            for g_ in gens.values():
                for _ in g_: pass
        def startup_iter(it, kind):
            @pl.when(it < 14)
            def _():
                for cq in w_copies(it + 2): cq.start()
            if kind == 0:
                @pl.when(it == 1)
                def _():
                    for cq in in_copies(1, 1): cq.start()
                @pl.when(it >= 2)
                def _():
                    wo_copy(it - 2).start()
            elif kind == 1:
                @pl.when(it == 9)
                def _():
                    wo_copy(7).start()
                @pl.when((it >= 10) & (it < 13))
                def _():
                    x_copy(it - 9).start()
            for cq in w_copies(it): cq.wait()
            if kind == 0:
                run_plan(splanA, {"p": proj_gen(it), "b1": stage1_gen(0, 0, it - 1)})
            else:
                run_plan([], {"p": proj_gen(it)})
        x_copy(0).wait()
        if staged:
            for cq in w_copies(0): cq.wait()
            for cq in w_copies(1): cq.start()
            for cq in in_copies(0, 0): cq.start()
            run_plan([], {"p": proj_gen(0)})
            for cq in w_copies(2): cq.start()
        else:
            startup_iter(0, -1)
        for cq in in_copies(0, 0): cq.wait()
        def loop_a(it, c):
            startup_iter(it, 0); return c
        jax.lax.fori_loop(1, 9, loop_a, 0, unroll=ua)
        def loop_b(it, c):
            startup_iter(it, 1); return c
        jax.lax.fori_loop(9, 16, loop_b, 0, unroll=ub)
        for part in range(8): wo_copy(part).wait()
        for part in range(1, 4): x_copy(part).wait()

        ri = jax.lax.broadcasted_iota(jnp.int32, (L, L), 0)
        ci = jax.lax.broadcasted_iota(jnp.int32, (L, L), 1)
        mask = (ri < M) | (ri >= ci)

        def slot_body(sg, mem):
            p = sg % 2
            j1 = jnp.minimum(sg + 1, 7)
            @pl.when(sg < NSL - 1)
            def _():
                for cq in in_copies(sg + 1, 1 - p): cq.wait()
            @pl.when(sg >= 1)
            def _():
                q_copy(sg - 1, 1 - p).wait()
            @pl.when(sg < NSL - 2)
            def _():
                for cq in in_copies(sg + 2, p): cq.start()
            q_copy(sg, p).start()
            if slotdma:
                @pl.when(sg >= 2)
                def _():
                    outa_slot_copy(0, p).wait()
                @pl.when(sg >= 3)
                def _():
                    outb_slot_copy(0, 1 - p).wait()
            def step(i, mem):
                s = sg * 8 + i
                par = i % 2
                if not slotdma:
                    outa_copy(0, par).wait()
                    out_copy(0, 0, par).wait()
                xr0 = pl.multiple_of(P0 + s * TS, 8)
                wr0 = pl.multiple_of(jax.lax.rem(s * TS, RING), 8)
                rr0 = pl.multiple_of(jax.lax.rem(s * SEG + 64, RING), 32)
                xs = xv[pl.ds(xr0, TS), :].astype(jnp.float32)
                h = jnp.concatenate([mem, xs], axis=0).astype(jnp.bfloat16)
                gens = {"b1": stage1_gen(j1, 1 - p, i), "b2": stage2_gen(p, i), "b3": stage3_gen(1 - p, i, par)}
                gens = {k_: v_ for k_, v_ in gens.items() if k_ in bsel}
                st = dict(ys={}, ps={}, outs={}, y=None)
                def do(op, t):
                    if op == "mm":
                        w = pltpu.bitcast(wqkv[:, t * G * 384:(t + 1) * G * 384], jnp.bfloat16)
                        st["ys"][t] = _dot(h, w)
                    elif op == "st":
                        ring[pl.ds(wr0, TS), t * G * 384:(t + 1) * G * 384] = st["ys"][t][M:, :]
                    elif op == "qk":
                        if noatt == 1: return
                        y = st["ys"][t]; pl_ = []
                        for ii in range(G):
                            c = (t * G + ii) * 384
                            q = jnp.concatenate([y[:M, ii * 384:ii * 384 + 128], ring[pl.ds(rr0, SEG), c:c + 128]], 0)
                            k = jnp.concatenate([y[:M, ii * 384 + 128:ii * 384 + 256], ring[pl.ds(rr0, SEG), c + 128:c + 256]], 0)
                            if noatt == 2:
                                pl_.append((_dot(q, k, NT), None)); continue
                            sc = jnp.where(mask, _dot(q, k, NT), -1e30)
                            m = jnp.max(sc, axis=1, keepdims=True)
                            e = jnp.exp2((sc - m) * (scale * LOG2E))
                            l = jnp.sum(e, axis=1, keepdims=True)
                            r = pltpu.reciprocal(l, approx=True)
                            r = r * (2.0 - l * r)
                            pl_.append((e, r) if smx == 1 else (e * r, None))
                        st["ps"][t] = pl_
                    elif op == "pv":
                        y = st["ys"][t]; ol = []
                        for ii in range(G):
                            c = (t * G + ii) * 384
                            v = jnp.concatenate([y[:M, ii * 384 + 256:ii * 384 + 384], ring[pl.ds(rr0, SEG), c + 256:c + 384]], 0)
                            if noatt == 1:
                                ol.append(v); continue
                            pp, rr_ = st["ps"][t][ii]
                            oo = _dot(pp, v)
                            ol.append(oo if rr_ is None else oo * rr_)
                        st["outs"][t] = ol
                    elif op == "wo":
                        t0, t1 = t
                        o = jnp.concatenate([oo for tt in range(t0, t1) for oo in st["outs"][tt]], axis=1)
                        wo = pltpu.bitcast(wo32[t0 * G * 64:t1 * G * 64, :], jnp.bfloat16)
                        yy = _dot(o, wo)
                        st["y"] = yy if st["y"] is None else st["y"] + yy
                    elif op in gens:
                        if doB:
                            for _ in range(t): next(gens[op], None)
                if scopes:
                    groups = []
                    for op, t in plan(NG):
                        if op in scopes or not groups: groups.append([])
                        groups[-1].append((op, t))
                    for gi, g_ in enumerate(groups):
                        with jax.named_scope("g%02d" % gi):
                            for op, t in g_: do(op, t)
                else:
                    for op, t in plan(NG):
                        do(op, t)
                if doB:
                    for g_ in gens.values():
                        for _ in g_: pass
                y = st["y"]
                mem = y[:M, :]
                if slotdma:
                    ostaS[p, pl.ds(pl.multiple_of(i * SEG, SEG), SEG), :] = y[M:, :].astype(jnp.bfloat16)
                    return mem
                osta[par] = y[M:, :].astype(jnp.bfloat16)
                outa_copy(s, par).start()
                @pl.when(sg >= 1)
                def _():
                    out_copy(sg - 1, i, par).start()
                @pl.when(sg == 0)
                def _():
                    pltpu.make_async_copy(ost.at[par], dummy_b.at[par], osem.at[par]).start()
                return mem
            mem = jax.lax.fori_loop(0, 8, step, mem, unroll=unroll)
            if slotdma:
                outa_slot_copy(sg, p).start()
                @pl.when(sg >= 1)
                def _():
                    outb_slot_copy(sg - 1, 1 - p).start()
            return mem
        mem = mem0v[...].astype(jnp.float32)
        jax.lax.fori_loop(0, NSL, slot_body, mem)
        jl = NSL - 1
        q_copy(jl, jl % 2).wait()
        if slotdma:
            outb_slot_copy(0, jl % 2).wait()
            def epi(i, c):
                for _ in stage3_gen(jl % 2, i, 0): pass
                return c
            jax.lax.fori_loop(0, 8, epi, 0)
            outb_slot_copy(jl, jl % 2).start()
            for par in range(2):
                outa_slot_copy(0, par).wait()
                outb_slot_copy(0, par).wait()
        else:
            def epi(i, c):
                par = i % 2
                out_copy(0, 0, par).wait()
                for _ in stage3_gen(jl % 2, i, par): pass
                out_copy(jl, i, par).start()
                return c
            jax.lax.fori_loop(0, 8, epi, 0)
            for par in range(2):
                outa_copy(0, par).wait()
                out_copy(0, 0, par).wait()

    def fn(x, mem0, wq, wk, wv, wo, q, k, v, shift_k, ssm_k, ssm_D):
        F, G_ = dft_consts()
        any_ = pl.BlockSpec(memory_space=pl.ANY)
        VM = pltpu.VMEM
        wq2, wk2, wv2 = [w.reshape(DM // 2, 2, H, DH) for w in (wq, wk, wv)]
        out = pl.pallas_call(
            kern, out_shape=jax.ShapeDtypeStruct((S, 2 * D), jnp.bfloat16),
            in_specs=[any_] * 14, out_specs=any_,
            scratch_shapes=[
                VM((S, DM), jnp.bfloat16), VM((3, 6, 512, 128), jnp.uint32),
                VM((DM // 2, H * 384), jnp.uint32), VM((H * DH // 2, DM), jnp.uint32),
                VM((RING, H * 384), jnp.float32), VM((2, SEG, DM), jnp.bfloat16),
                VM((M, DM), jnp.bfloat16), VM((4, D), jnp.bfloat16), VM((D,), jnp.bfloat16),
                VM((256, 128), jnp.bfloat16), VM((128, 256), jnp.bfloat16),
                VM((2, S, 128), jnp.bfloat16), VM((2, S, 128), jnp.bfloat16),
                VM((2, 128, S), jnp.bfloat16), VM((2, S, 128), jnp.bfloat16),
                VM((S + 8, 128), jnp.float32),
                VM((2, 16, 256, 128), jnp.float32), VM((2, 16, 256, 128), jnp.float32), VM((2, 16, 256, 128), jnp.float32),
                VM((256, 128), jnp.float32), VM((8, D), jnp.float32),
                VM((2, 256, 128), jnp.bfloat16), VM((2, SEG, DM), jnp.bfloat16), VM((2, 256, 128), jnp.bfloat16),
                VM((2, 256, DM), jnp.bfloat16), VM((2, S, 128), jnp.bfloat16), VM((2, S, 128), jnp.bfloat16),
                pltpu.SemaphoreType.DMA((3,)), pltpu.SemaphoreType.DMA((4,)), pltpu.SemaphoreType.DMA,
                pltpu.SemaphoreType.DMA((5,)), pltpu.SemaphoreType.DMA((2,)),
                pltpu.SemaphoreType.DMA((2, 3)), pltpu.SemaphoreType.DMA((2,)), pltpu.SemaphoreType.DMA((2,))],
            compiler_params=pltpu.CompilerParams(vmem_limit_bytes=120 * 1024 * 1024),
        )(x.reshape(S, DM), mem0.reshape(M, DM), wq2, wk2, wv2, wo.reshape(H * DH, DM),
          q.reshape(S, D), k.reshape(S, D), v.reshape(S, D), shift_k.T, ssm_k, ssm_D,
          jnp.asarray(F, jnp.bfloat16), jnp.asarray(G_, jnp.bfloat16))
        return out.reshape(1, S, 2 * D)
    return fn


@jax.jit
def pallas_concat_heads__memory_aug_recurrent_mem_tr__ssm_conv_h3__prompt_kernel(
    A_x, A_mem0, A_Wq, A_Wk, A_Wv, A_Wo, A_seg_len, B_q, B_k, B_v, B_shift_k, B_ssm_k, B_ssm_D,
):
    return make()(A_x, A_mem0, A_Wq, A_Wk, A_Wv, A_Wo, B_q, B_k, B_v, B_shift_k, B_ssm_k, B_ssm_D)
```

```python
import jax
import jax.numpy as jnp
import numpy as np
from jax.experimental import pallas as pl
from jax.experimental.pallas import tpu as pltpu

S, DM, H, DH, M, SEG = 2048, 1024, 32, 128, 8, 32
D = 1024
L = M + SEG
P0 = 512
TS = 24
RING = 576
G = 4
NG = H // G
NB = D // 128
NT = (((1,), (1,)), ((), ()))
NN = (((1,), (0,)), ((), ()))


def _dot(a, b, dims=NN):
    return jax.lax.dot_general(a, b, dims, preferred_element_type=jnp.float32)


def _dft_consts():
    n, c = 256, 128
    f = np.concatenate([np.arange(0, 128, 2), np.arange(1, 128, 2)])
    th = 2 * np.pi * np.outer(f + 0.5, np.arange(c)) / n
    fwd = np.concatenate([np.cos(th), -np.sin(th)], 0)
    inv = np.concatenate([np.cos(th).T, -np.sin(th).T], 1) * (2.0 / n)
    return fwd.astype(np.float32), inv.astype(np.float32)


def _step_plan():
    pre = {0: ["b1", "b1", "b2", "b2"], 1: ["b2"], 2: ["b2", "b1"], 3: ["b1", "b2"],
           4: ["b2", "b2", "b2"], 9: ["b3", "b3"]}
    lag_s, lag_p, split_t, split_g = 1, 3, 10, 5
    plan = []
    for t in range(NG + lag_p):
        if t < NG:
            plan.append(("mm", t))
        if 0 <= t - lag_s < NG:
            plan += [("st", t - lag_s), ("qk", t - lag_s)]
        if 0 <= t - lag_p < NG:
            plan.append(("pv", t - lag_p))
        if t == split_t:
            plan.append(("wo", (0, split_g)))
        plan += [(b, 1) for b in pre.get(t, [])]
    plan.append(("wo", (split_g, NG)))
    return plan


def _kernel(x_hbm, mem0_hbm, wq_hbm, wk_hbm, wv_hbm, wo_hbm,
            q_hbm, k_hbm, v_hbm, sk_hbm, w_hbm, dd_hbm, f_hbm, g_hbm,
            out_hbm,
            xv, raw, wqkv, wo32, ring, osta, mem0v, skv, ddv, fv, gv,
            kin, vin, win, qin, uh, whp, yh, wprev, ost, skt,
            wsem, xsem, wosem, smsem, osema, isem, qsem, osem):
    f32, bf16, u32 = jnp.float32, jnp.bfloat16, jnp.uint32

    def in_copies(j, p):
        c = pl.multiple_of(j * 128, 128)
        return [pltpu.make_async_copy(k_hbm.at[:, pl.ds(c, 128)], kin.at[p], isem.at[p, 0]),
                pltpu.make_async_copy(v_hbm.at[:, pl.ds(c, 128)], vin.at[p], isem.at[p, 1]),
                pltpu.make_async_copy(w_hbm.at[pl.ds(c, 128), :], win.at[p], isem.at[p, 2])]

    def q_copy(j, p):
        c = pl.multiple_of(j * 128, 128)
        return pltpu.make_async_copy(q_hbm.at[:, pl.ds(c, 128)], qin.at[p], qsem.at[p])

    def outa_copy(sg, p):
        r = pl.multiple_of(sg * 256, 256)
        return pltpu.make_async_copy(osta.at[p], out_hbm.at[pl.ds(r, 256), pl.ds(0, DM)], osema.at[p])

    def outb_copy(j, p):
        c = pl.multiple_of(D + j * 128, 128)
        return pltpu.make_async_copy(ost.at[p], out_hbm.at[:, pl.ds(c, 128)], osem.at[p])

    wsrc = [w.bitcast(u32) for w in (wq_hbm, wk_hbm, wv_hbm)]

    def w_copies(hp):
        slot = hp % 3
        return [pltpu.make_async_copy(wsrc[j].at[:, par, hp, :], raw.at[slot, 2 * j + par], wsem.at[slot])
                for j in range(3) for par in range(2)]

    def wo_copy(part):
        r = pl.multiple_of(part * 512, 512)
        return pltpu.make_async_copy(wo_hbm.at[pl.ds(r, 512), :],
                                     wo32.bitcast(bf16).at[pl.ds(r, 512), :], wosem)

    def x_copy(part):
        r = pl.multiple_of(part * 512, 512)
        return pltpu.make_async_copy(x_hbm.at[pl.ds(r, 512), :], xv.at[pl.ds(r, 512), :], xsem.at[part])

    small = [pltpu.make_async_copy(a, b, smsem.at[n]) for n, (a, b) in enumerate(
        ((mem0_hbm, mem0v), (sk_hbm, skv), (dd_hbm, ddv), (f_hbm, fv), (g_hbm, gv)))]

    def stage1(j, p, i):
        c0 = pl.multiple_of(j * 128, 128)
        taps = skt[:, pl.ds(c0, 128)]
        dvec = taps[4:5]
        first = i == 0
        prev = jnp.where(first, 0.0, wprev[...])
        kf_prev = None
        for c in range(2):
            rc = pl.multiple_of(i * 256 + c * 128, 128)
            a = 2 * i + c
            kf = kin[p, pl.ds(rc, 128), :].astype(f32)
            if c == 0:
                rp = pl.multiple_of(jnp.maximum(rc - 8, 0), 8)
                tail = jnp.where(first, 0.0, kin[p, pl.ds(rp, 8), :].astype(f32))
            else:
                tail = kf_prev[120:128]
            ext = jnp.concatenate([tail, kf], axis=0)
            ks = (kf * taps[0:1] + ext[7:135] * taps[1:2]
                  + ext[6:134] * taps[2:3] + ext[5:133] * taps[3:4])
            kf_prev = kf
            kv = ks * vin[p, pl.ds(rc, 128), :].astype(f32)
            uh[p, a] = _dot(fv[...], kv)
            yield
            wt = win[p, :, pl.ds(pl.multiple_of(a * 128, 128), 128)]
            wh = _dot(fv[...], wt, NT)
            pr, pi_ = prev[:128], prev[128:]
            re = jnp.concatenate([wh[0:64] - pi_[0:64], wh[64:128] + pi_[64:128]], 0)
            im = jnp.concatenate([wh[128:192] + pr[0:64], wh[192:256] - pr[64:128]], 0)
            if c == 0:
                re = re + jnp.where(first, dvec, 0.0)
            whp[p, a, 0:128] = re
            whp[p, a, 128:256] = im
            prev = wh
            yield
        wprev[...] = prev

    def stage2(p, i):
        ob = 4
        for gg in range(2):
            rr = pl.multiple_of(i * 16 + gg * 8, 8)
            ri = pl.multiple_of(128 + i * 16 + gg * 8, 8)
            for b in range(16 // ob):
                outs = list(range(b * ob, (b + 1) * ob))
                accr, acci, wc = {}, {}, {}
                for ap in range(outs[-1] + 1):
                    ur = uh[p, ap, pl.ds(rr, 8), :]
                    ui = uh[p, ap, pl.ds(ri, 8), :]
                    for a in outs:
                        m = a - ap
                        if m < 0:
                            continue
                        if m not in wc:
                            wc[m] = (whp[p, m, pl.ds(rr, 8), :], whp[p, m, pl.ds(ri, 8), :])
                        wr, wi = wc[m]
                        tr = ur * wr - ui * wi
                        ti = ur * wi + ui * wr
                        accr[a] = tr if a not in accr else accr[a] + tr
                        acci[a] = ti if a not in acci else acci[a] + ti
                for a in outs:
                    yh[p, a, pl.ds(rr, 8), :] = accr[a]
                    yh[p, a, pl.ds(ri, 8), :] = acci[a]
                yield

    def stage3(p, i):
        for c in range(2):
            a = 2 * i + c
            y = _dot(gv[...], yh[p, a])
            r = pl.multiple_of(a * 128, 128)
            ost[p, pl.ds(r, 128), :] = (qin[p, pl.ds(r, 128), :].astype(f32) * y).astype(bf16)
            yield

    def drain(*gens):
        for g in gens:
            for _ in g:
                pass

    def project(hp):
        slot = hp % 3
        lo, hi = [], []
        for j in range(3):
            ev, od = raw[slot, 2 * j], raw[slot, 2 * j + 1]
            lo.append((ev & u32(0xFFFF)) | (od << 16))
            hi.append((ev >> 16) | (od & u32(0xFFFF0000)))
        w32 = jnp.concatenate(lo + hi, axis=1)
        c0 = pl.multiple_of(hp * 768, 768)
        wqkv[:, pl.ds(c0, 768)] = w32
        w = pltpu.bitcast(w32, bf16)
        for rb in range(P0 // 256):
            ring[pl.ds(64 + rb * 256, 256), pl.ds(c0, 768)] = _dot(xv[rb * 256:(rb + 1) * 256, :], w)

    x_copy(0).start()
    for cp in w_copies(0):
        cp.start()
    for cp in small:
        cp.start()
    yh[1] = jnp.zeros((16, 256, 128), f32)
    qin[1] = jnp.zeros((S, 128), bf16)
    wprev[...] = jnp.zeros((256, 128), f32)
    for cp in small:
        cp.wait()
    skt[0:4, :] = skv[...].astype(f32)
    skt[4:5, :] = ddv[...].astype(f32).reshape(1, D)
    skt[5:8, :] = jnp.zeros((3, D), f32)
    x_copy(0).wait()
    for cp in w_copies(0):
        cp.wait()
    for cp in w_copies(1):
        cp.start()
    for cp in in_copies(0, 0):
        cp.start()
    project(0)
    for cp in w_copies(2):
        cp.start()
    for cp in in_copies(0, 0):
        cp.wait()

    def startup_a(it, carry):
        for cp in w_copies(it):
            cp.wait()
        project(it)
        drain(stage1(0, 0, it - 1))
        for cp in w_copies(it + 2):
            cp.start()

        @pl.when(it == 1)
        def _():
            for cp in in_copies(1, 1):
                cp.start()

        @pl.when(it >= 2)
        def _():
            wo_copy(it - 2).start()
        return carry

    def startup_b(it, carry):
        for cp in w_copies(it):
            cp.wait()
        project(it)

        @pl.when(it < 14)
        def _():
            for cp in w_copies(it + 2):
                cp.start()

        @pl.when(it == 9)
        def _():
            wo_copy(7).start()

        @pl.when((it >= 10) & (it < 13))
        def _():
            x_copy(it - 9).start()
        return carry

    jax.lax.fori_loop(1, 9, startup_a, 0)
    jax.lax.fori_loop(9, 16, startup_b, 0)
    for part in range(8):
        wo_copy(part).wait()
    for part in range(1, 4):
        x_copy(part).wait()

    rows = jax.lax.broadcasted_iota(jnp.int32, (L, L), 0)
    cols = jax.lax.broadcasted_iota(jnp.int32, (L, L), 1)
    mask = (rows < M) | (rows >= cols)
    exp_scale = float(DH ** -0.5 * np.log2(np.e))
    plan = _step_plan()

    def slot_body(sg, mem):
        p = sg % 2

        @pl.when(sg < NB - 1)
        def _():
            for cp in in_copies(sg + 1, 1 - p):
                cp.wait()

        @pl.when(sg >= 1)
        def _():
            q_copy(sg - 1, 1 - p).wait()

        @pl.when(sg < NB - 2)
        def _():
            for cp in in_copies(sg + 2, p):
                cp.start()
        q_copy(sg, p).start()

        @pl.when(sg >= 2)
        def _():
            outa_copy(0, p).wait()

        @pl.when(sg >= 3)
        def _():
            outb_copy(0, 1 - p).wait()

        def step(i, mem):
            s = sg * 8 + i
            xr = pl.multiple_of(P0 + s * TS, 8)
            wr = pl.multiple_of(jax.lax.rem(s * TS, RING), 8)
            rd = pl.multiple_of(jax.lax.rem(s * SEG + 64, RING), 32)
            h = jnp.concatenate([mem, xv[pl.ds(xr, TS), :].astype(f32)], axis=0).astype(bf16)
            gens = {"b1": stage1(jnp.minimum(sg + 1, NB - 1), 1 - p, i),
                    "b2": stage2(p, i),
                    "b3": stage3(1 - p, i)}
            ys, ps, outs, y = {}, {}, {}, None

            def operand(t, ii, j):
                c = ii * 384 + j * 128
                return jnp.concatenate(
                    [ys[t][:M, c:c + 128], ring[pl.ds(rd, SEG), t * G * 384 + c:t * G * 384 + c + 128]], 0)

            for op, t in plan:
                if op == "mm":
                    w = pltpu.bitcast(wqkv[:, t * G * 384:(t + 1) * G * 384], bf16)
                    ys[t] = _dot(h, w)
                elif op == "st":
                    ring[pl.ds(wr, TS), t * G * 384:(t + 1) * G * 384] = ys[t][M:, :]
                elif op == "qk":
                    ps[t] = []
                    for ii in range(G):
                        sc = jnp.where(mask, _dot(operand(t, ii, 0), operand(t, ii, 1), NT), -1e30)
                        e = jnp.exp2((sc - jnp.max(sc, axis=1, keepdims=True)) * exp_scale)
                        l = jnp.sum(e, axis=1, keepdims=True)
                        r = pltpu.reciprocal(l, approx=True)
                        ps[t].append((e, r * (2.0 - l * r)))
                elif op == "pv":
                    outs[t] = [_dot(ps[t][ii][0], operand(t, ii, 2)) * ps[t][ii][1] for ii in range(G)]
                elif op == "wo":
                    t0, t1 = t
                    o = jnp.concatenate([oo for tt in range(t0, t1) for oo in outs[tt]], axis=1)
                    yy = _dot(o, pltpu.bitcast(wo32[t0 * G * 64:t1 * G * 64, :], bf16))
                    y = yy if y is None else y + yy
                else:
                    next(gens[op], None)
            drain(*gens.values())
            osta[p, pl.ds(pl.multiple_of(i * SEG, SEG), SEG), :] = y[M:, :].astype(bf16)
            return y[:M, :]

        mem = jax.lax.fori_loop(0, 8, step, mem, unroll=4)
        outa_copy(sg, p).start()

        @pl.when(sg >= 1)
        def _():
            outb_copy(sg - 1, 1 - p).start()
        return mem

    jax.lax.fori_loop(0, NB, slot_body, mem0v[...].astype(f32))

    jl = NB - 1
    q_copy(jl, jl % 2).wait()
    outb_copy(0, jl % 2).wait()

    def epilogue(i, carry):
        drain(stage3(jl % 2, i))
        return carry
    jax.lax.fori_loop(0, 8, epilogue, 0)
    outb_copy(jl, jl % 2).start()
    for p in range(2):
        outa_copy(0, p).wait()
        outb_copy(0, p).wait()


def make():
    def fn(x, mem0, wq, wk, wv, wo, q, k, v, shift_k, ssm_k, ssm_d):
        fwd, inv = _dft_consts()
        any_ = pl.BlockSpec(memory_space=pl.ANY)
        vm, dma = pltpu.VMEM, pltpu.SemaphoreType.DMA
        f32, bf16, u32 = jnp.float32, jnp.bfloat16, jnp.uint32
        out = pl.pallas_call(
            _kernel,
            out_shape=jax.ShapeDtypeStruct((S, 2 * D), bf16),
            in_specs=[any_] * 14,
            out_specs=any_,
            scratch_shapes=[
                vm((S, DM), bf16), vm((3, 6, DM // 2, 128), u32),
                vm((DM // 2, H * 384), u32), vm((H * DH // 2, DM), u32),
                vm((RING, H * 384), f32), vm((2, 256, DM), bf16),
                vm((M, DM), bf16), vm((4, D), bf16), vm((D,), bf16),
                vm((256, 128), bf16), vm((128, 256), bf16),
                vm((2, S, 128), bf16), vm((2, S, 128), bf16), vm((2, 128, S), bf16), vm((2, S, 128), bf16),
                vm((2, 16, 256, 128), f32), vm((2, 16, 256, 128), f32), vm((2, 16, 256, 128), f32),
                vm((256, 128), f32), vm((2, S, 128), bf16), vm((8, D), f32),
                dma((3,)), dma((4,)), dma, dma((5,)), dma((2,)), dma((2, 3)), dma((2,)), dma((2,))],
            compiler_params=pltpu.CompilerParams(
                vmem_limit_bytes=120 * 1024 * 1024,
                flags={"XLA_TPU_EVENLY_DISTRIBUTE_CRITICAL_NODES": True},
                disable_bounds_checks=NOBOUNDS),
        )(x.reshape(S, DM), mem0.reshape(M, DM),
          wq.reshape(DM // 2, 2, H, DH), wk.reshape(DM // 2, 2, H, DH), wv.reshape(DM // 2, 2, H, DH),
          wo.reshape(H * DH, DM), q.reshape(S, D), k.reshape(S, D), v.reshape(S, D),
          shift_k.T, ssm_k, ssm_d, jnp.asarray(fwd, bf16), jnp.asarray(inv, bf16))
        return out.reshape(1, S, 2 * D)
    return fn


NOBOUNDS = True


@jax.jit
def pallas_concat_heads__memory_aug_recurrent_mem_tr__ssm_conv_h3__prompt_kernel(
    A_x, A_mem0, A_Wq, A_Wk, A_Wv, A_Wo, A_seg_len, B_q, B_k, B_v, B_shift_k, B_ssm_k, B_ssm_D,
):
    return make()(A_x, A_mem0, A_Wq, A_Wk, A_Wv, A_Wo, B_q, B_k, B_v, B_shift_k, B_ssm_k, B_ssm_D)
```

```python
import jax
import jax.numpy as jnp
import numpy as np
from jax.experimental import pallas as pl
from jax.experimental.pallas import tpu as pltpu

S, DM, H, DH, M, SEG = 2048, 1024, 32, 128, 8, 32
D = 1024
L = M + SEG
P0 = 512
TS = 24
RING = 576
G = 4
NG = H // G
NB = D // 128
NT = (((1,), (1,)), ((), ()))
NN = (((1,), (0,)), ((), ()))


def _dot(a, b, dims=NN):
    return jax.lax.dot_general(a, b, dims, preferred_element_type=jnp.float32)


def _dft_consts():
    n, c = 256, 128
    f = np.concatenate([np.arange(0, 128, 2), np.arange(1, 128, 2)])
    th = 2 * np.pi * np.outer(f + 0.5, np.arange(c)) / n
    fwd = np.concatenate([np.cos(th), -np.sin(th)], 0)
    inv = np.concatenate([np.cos(th).T, -np.sin(th).T], 1) * (2.0 / n)
    return fwd.astype(np.float32), inv.astype(np.float32)


def _step_plan():
    pre = {0: ["b1", "b1", "b2", "b2"], 1: ["b2"], 2: ["b2", "b1"], 3: ["b1", "b2"],
           4: ["b2", "b2", "b2"], 9: ["b3", "b3"]}
    lag_s, lag_p, split_t, split_g = 1, 3, 10, 5
    plan = []
    for t in range(NG + lag_p):
        if t < NG:
            plan.append(("mm", t))
        if 0 <= t - lag_s < NG:
            plan += [("st", t - lag_s), ("qk", t - lag_s)]
        if 0 <= t - lag_p < NG:
            plan.append(("pv", t - lag_p))
        if t == split_t:
            plan.append(("wo", (0, split_g)))
        plan += [(b, 1) for b in pre.get(t, [])]
    plan.append(("wo", (split_g, NG)))
    return plan


def _kernel(x_hbm, mem0_hbm, wq_hbm, wk_hbm, wv_hbm, wo_hbm,
            q_hbm, k_hbm, v_hbm, sk_hbm, w_hbm, dd_hbm, f_hbm, g_hbm,
            out_hbm,
            xv, raw, wqkv, wo32, ring, osta, mem0v, skv, ddv, fv, gv,
            kin, vin, win, qin, uh, whp, yh, wprev, ost, skt,
            w0sem, wsem, xsem, wosem, smsem, osema, isem, qsem, osem):
    f32, bf16, u32 = jnp.float32, jnp.bfloat16, jnp.uint32

    def in_copies(j, p):
        c = pl.multiple_of(j * 128, 128)
        return [pltpu.make_async_copy(k_hbm.at[:, pl.ds(c, 128)], kin.at[p], isem.at[p, 0]),
                pltpu.make_async_copy(v_hbm.at[:, pl.ds(c, 128)], vin.at[p], isem.at[p, 1]),
                pltpu.make_async_copy(w_hbm.at[pl.ds(c, 128), :], win.at[p], isem.at[p, 2])]

    def q_copy(j, p):
        c = pl.multiple_of(j * 128, 128)
        return pltpu.make_async_copy(q_hbm.at[:, pl.ds(c, 128)], qin.at[p], qsem.at[p])

    def outa_copy(sg, p):
        r = pl.multiple_of(sg * 256, 256)
        return pltpu.make_async_copy(osta.at[p], out_hbm.at[pl.ds(r, 256), pl.ds(0, DM)], osema.at[p])

    def outb_copy(j, p):
        c = pl.multiple_of(D + j * 128, 128)
        return pltpu.make_async_copy(ost.at[p], out_hbm.at[:, pl.ds(c, 128)], osem.at[p])

    wsrc = [w.bitcast(u32) for w in (wq_hbm, wk_hbm, wv_hbm)]

    def w_copies(hp):
        slot = hp % 3
        return [pltpu.make_async_copy(wsrc[j].at[:, par, hp, :], raw.at[slot, 2 * j + par], wsem.at[slot])
                for j in range(3) for par in range(2)]

    def wo_copy(part):
        r = pl.multiple_of(part * 512, 512)
        return pltpu.make_async_copy(wo_hbm.at[pl.ds(r, 512), :],
                                     wo32.bitcast(bf16).at[pl.ds(r, 512), :], wosem)

    def x_copy(part):
        r = pl.multiple_of(part * 512, 512)
        return pltpu.make_async_copy(x_hbm.at[pl.ds(r, 512), :], xv.at[pl.ds(r, 512), :], xsem.at[part + 1])

    small = [pltpu.make_async_copy(a, b, smsem.at[n]) for n, (a, b) in enumerate(
        ((mem0_hbm, mem0v), (sk_hbm, skv), (dd_hbm, ddv), (f_hbm, fv), (g_hbm, gv)))]

    def stage1(j, p, i):
        c0 = pl.multiple_of(j * 128, 128)
        taps = skt[:, pl.ds(c0, 128)]
        dvec = taps[4:5]
        first = i == 0
        prev = jnp.where(first, 0.0, wprev[...])
        kf_prev = None
        for c in range(2):
            rc = pl.multiple_of(i * 256 + c * 128, 128)
            a = 2 * i + c
            kf = kin[p, pl.ds(rc, 128), :].astype(f32)
            if c == 0:
                rp = pl.multiple_of(jnp.maximum(rc - 8, 0), 8)
                tail = jnp.where(first, 0.0, kin[p, pl.ds(rp, 8), :].astype(f32))
            else:
                tail = kf_prev[120:128]
            ext = jnp.concatenate([tail, kf], axis=0)
            ks = (kf * taps[0:1] + ext[7:135] * taps[1:2]
                  + ext[6:134] * taps[2:3] + ext[5:133] * taps[3:4])
            kf_prev = kf
            kv = ks * vin[p, pl.ds(rc, 128), :].astype(f32)
            uh[p, a] = _dot(fv[...], kv)
            yield
            wt = win[p, :, pl.ds(pl.multiple_of(a * 128, 128), 128)]
            wh = _dot(fv[...], wt, NT)
            pr, pi_ = prev[:128], prev[128:]
            re = jnp.concatenate([wh[0:64] - pi_[0:64], wh[64:128] + pi_[64:128]], 0)
            im = jnp.concatenate([wh[128:192] + pr[0:64], wh[192:256] - pr[64:128]], 0)
            if c == 0:
                re = re + jnp.where(first, dvec, 0.0)
            whp[p, a, 0:128] = re
            whp[p, a, 128:256] = im
            prev = wh
            yield
        wprev[...] = prev

    def stage2(p, i):
        ob = 4
        for gg in range(2):
            rr = pl.multiple_of(i * 16 + gg * 8, 8)
            ri = pl.multiple_of(128 + i * 16 + gg * 8, 8)
            for b in range(16 // ob):
                outs = list(range(b * ob, (b + 1) * ob))
                accr, acci, wc = {}, {}, {}
                for ap in range(outs[-1] + 1):
                    ur = uh[p, ap, pl.ds(rr, 8), :]
                    ui = uh[p, ap, pl.ds(ri, 8), :]
                    for a in outs:
                        m = a - ap
                        if m < 0:
                            continue
                        if m not in wc:
                            wc[m] = (whp[p, m, pl.ds(rr, 8), :], whp[p, m, pl.ds(ri, 8), :])
                        wr, wi = wc[m]
                        tr = ur * wr - ui * wi
                        ti = ur * wi + ui * wr
                        accr[a] = tr if a not in accr else accr[a] + tr
                        acci[a] = ti if a not in acci else acci[a] + ti
                for a in outs:
                    yh[p, a, pl.ds(rr, 8), :] = accr[a]
                    yh[p, a, pl.ds(ri, 8), :] = acci[a]
                yield

    def stage3(p, i):
        for c in range(2):
            a = 2 * i + c
            y = _dot(gv[...], yh[p, a])
            r = pl.multiple_of(a * 128, 128)
            ost[p, pl.ds(r, 128), :] = (qin[p, pl.ds(r, 128), :].astype(f32) * y).astype(bf16)
            yield

    def drain(*gens):
        for g in gens:
            for _ in g:
                pass

    def project(hp):
        slot = hp % 3
        lo, hi = [], []
        for j in range(3):
            ev, od = raw[slot, 2 * j], raw[slot, 2 * j + 1]
            lo.append((ev & u32(0xFFFF)) | (od << 16))
            hi.append((ev >> 16) | (od & u32(0xFFFF0000)))
        w32 = jnp.concatenate(lo + hi, axis=1)
        c0 = pl.multiple_of(hp * 768, 768)
        wqkv[:, pl.ds(c0, 768)] = w32
        w = pltpu.bitcast(w32, bf16)
        for rb in range(P0 // 256):
            ring[pl.ds(64 + rb * 256, 256), pl.ds(c0, 768)] = _dot(xv[rb * 256:(rb + 1) * 256, :], w)

    w0 = [[pltpu.make_async_copy(wsrc[j].at[:, par, 0, :], raw.at[0, 2 * j + par], w0sem.at[j]) for par in range(2)]
          for j in range(3)]
    xh = [pltpu.make_async_copy(x_hbm.at[pl.ds(r * 256, 256), :], xv.at[pl.ds(r * 256, 256), :], xsem.at[r])
          for r in range(2)]
    xh[0].start()
    for cp in w0[0]:
        cp.start()
    for cp in small:
        cp.start()
    for cp in w0[1] + w0[2]:
        cp.start()
    xh[1].start()
    yh[1] = jnp.zeros((16, 256, 128), f32)
    qin[1] = jnp.zeros((S, 128), bf16)
    wprev[...] = jnp.zeros((256, 128), f32)
    xh[0].wait()
    first_w = []
    for j in range(3):
        for cp in w0[j]:
            cp.wait()
        ev, od = raw[0, 2 * j], raw[0, 2 * j + 1]
        lo = (ev & u32(0xFFFF)) | (od << 16)
        hi = (ev >> 16) | (od & u32(0xFFFF0000))
        wqkv[:, j * 128:(j + 1) * 128] = lo
        wqkv[:, 384 + j * 128:384 + (j + 1) * 128] = hi
        w = pltpu.bitcast(jnp.concatenate([lo, hi], axis=1), bf16)
        first_w.append(w)
        y = _dot(xv[0:256, :], w)
        ring[64:320, j * 128:(j + 1) * 128] = y[:, :128]
        ring[64:320, 384 + j * 128:384 + (j + 1) * 128] = y[:, 128:]
        if j == 0:
            for cp in w_copies(1):
                cp.start()
    xh[1].wait()
    for j in range(3):
        y = _dot(xv[256:512, :], first_w[j])
        ring[320:576, j * 128:(j + 1) * 128] = y[:, :128]
        ring[320:576, 384 + j * 128:384 + (j + 1) * 128] = y[:, 128:]
    for cp in w_copies(2):
        cp.start()
    for cp in in_copies(0, 0):
        cp.start()
    for cp in small:
        cp.wait()
    skt[0:4, :] = skv[...].astype(f32)
    skt[4:5, :] = ddv[...].astype(f32).reshape(1, D)
    skt[5:8, :] = jnp.zeros((3, D), f32)

    def startup_1(it, carry):
        for cp in w_copies(it):
            cp.wait()
        project(it)
        for cp in w_copies(it + 2):
            cp.start()
        return carry
    startup_1(1, 0)
    for cp in in_copies(0, 0):
        cp.wait()

    def startup_a(it, carry):
        for cp in w_copies(it):
            cp.wait()
        project(it)
        drain(stage1(0, 0, it - 2))
        for cp in w_copies(it + 2):
            cp.start()

        @pl.when(it == 2)
        def _():
            for cp in in_copies(1, 1):
                cp.start()

        @pl.when(it >= 3)
        def _():
            wo_copy(it - 3).start()
        return carry

    def startup_b(it, carry):
        for cp in w_copies(it):
            cp.wait()
        project(it)

        @pl.when(it < 14)
        def _():
            for cp in w_copies(it + 2):
                cp.start()

        @pl.when(it == 10)
        def _():
            wo_copy(7).start()

        @pl.when((it >= 11) & (it < 14))
        def _():
            x_copy(it - 10).start()
        return carry

    jax.lax.fori_loop(2, 10, startup_a, 0)
    jax.lax.fori_loop(10, 16, startup_b, 0)
    for part in range(8):
        wo_copy(part).wait()
    for part in range(1, 4):
        x_copy(part).wait()

    rows = jax.lax.broadcasted_iota(jnp.int32, (L, L), 0)
    cols = jax.lax.broadcasted_iota(jnp.int32, (L, L), 1)
    mask = (rows < M) | (rows >= cols)
    exp_scale = float(DH ** -0.5 * np.log2(np.e))
    plan = _step_plan()

    def slot_body(sg, mem):
        p = sg % 2

        @pl.when(sg < NB - 1)
        def _():
            for cp in in_copies(sg + 1, 1 - p):
                cp.wait()

        @pl.when(sg >= 1)
        def _():
            q_copy(sg - 1, 1 - p).wait()

        @pl.when(sg < NB - 2)
        def _():
            for cp in in_copies(sg + 2, p):
                cp.start()
        q_copy(sg, p).start()

        @pl.when(sg >= 2)
        def _():
            outa_copy(0, p).wait()

        @pl.when(sg >= 3)
        def _():
            outb_copy(0, 1 - p).wait()

        def step(i, mem):
            s = sg * 8 + i
            xr = pl.multiple_of(P0 + s * TS, 8)
            wr = pl.multiple_of(jax.lax.rem(s * TS, RING), 8)
            rd = pl.multiple_of(jax.lax.rem(s * SEG + 64, RING), 32)
            h = jnp.concatenate([mem, xv[pl.ds(xr, TS), :].astype(f32)], axis=0).astype(bf16)
            gens = {"b1": stage1(jnp.minimum(sg + 1, NB - 1), 1 - p, i),
                    "b2": stage2(p, i),
                    "b3": stage3(1 - p, i)}
            ys, ps, outs, y = {}, {}, {}, None

            def operand(t, ii, j):
                c = ii * 384 + j * 128
                return jnp.concatenate(
                    [ys[t][:M, c:c + 128], ring[pl.ds(rd, SEG), t * G * 384 + c:t * G * 384 + c + 128]], 0)

            for op, t in plan:
                if op == "mm":
                    ys[t] = _dot(h, pltpu.bitcast(wqkv[:, t * G * 384:(t + 1) * G * 384], bf16))
                elif op == "st":
                    ring[pl.ds(wr, TS), t * G * 384:(t + 1) * G * 384] = ys[t][M:, :]
                elif op == "qk":
                    ps[t] = []
                    for ii in range(G):
                        sc = jnp.where(mask, _dot(operand(t, ii, 0), operand(t, ii, 1), NT), -1e30)
                        e = jnp.exp2((sc - jnp.max(sc, axis=1, keepdims=True)) * exp_scale)
                        l = jnp.sum(e, axis=1, keepdims=True)
                        r = pltpu.reciprocal(l, approx=True)
                        ps[t].append((e, r * (2.0 - l * r)))
                elif op == "pv":
                    outs[t] = [_dot(ps[t][ii][0], operand(t, ii, 2)) * ps[t][ii][1] for ii in range(G)]
                elif op == "wo":
                    t0, t1 = t
                    o = jnp.concatenate([oo for tt in range(t0, t1) for oo in outs[tt]], axis=1)
                    yy = _dot(o, pltpu.bitcast(wo32[t0 * G * 64:t1 * G * 64, :], bf16))
                    y = yy if y is None else y + yy
                else:
                    next(gens[op], None)
            drain(*gens.values())
            osta[p, pl.ds(pl.multiple_of(i * SEG, SEG), SEG), :] = y[M:, :].astype(bf16)
            return y[:M, :]

        mem = jax.lax.fori_loop(0, 8, step, mem, unroll=4)
        outa_copy(sg, p).start()

        @pl.when(sg >= 1)
        def _():
            outb_copy(sg - 1, 1 - p).start()
        return mem

    jax.lax.fori_loop(0, NB, slot_body, mem0v[...].astype(f32))

    jl = NB - 1
    q_copy(jl, jl % 2).wait()
    outb_copy(0, jl % 2).wait()

    def last_copy(i):
        r = pl.multiple_of(i * 256, 256)
        return pltpu.make_async_copy(ost.at[jl % 2, pl.ds(r, 256), :],
                                     out_hbm.at[pl.ds(r, 256), pl.ds(D + jl * 128, 128)], osem.at[jl % 2])

    def epilogue(i, carry):
        drain(stage3(jl % 2, i))
        last_copy(i).start()
        return carry
    jax.lax.fori_loop(0, 8, epilogue, 0)
    for p in range(2):
        outa_copy(0, p).wait()
    outb_copy(0, 1 - jl % 2).wait()
    for i in range(8):
        last_copy(i).wait()


def make():
    def fn(x, mem0, wq, wk, wv, wo, q, k, v, shift_k, ssm_k, ssm_d):
        fwd, inv = _dft_consts()
        any_ = pl.BlockSpec(memory_space=pl.ANY)
        vm, dma = pltpu.VMEM, pltpu.SemaphoreType.DMA
        f32, bf16, u32 = jnp.float32, jnp.bfloat16, jnp.uint32
        out = pl.pallas_call(
            _kernel,
            out_shape=jax.ShapeDtypeStruct((S, 2 * D), bf16),
            in_specs=[any_] * 14,
            out_specs=any_,
            scratch_shapes=[
                vm((S, DM), bf16), vm((3, 6, DM // 2, 128), u32),
                vm((DM // 2, H * 384), u32), vm((H * DH // 2, DM), u32),
                vm((RING, H * 384), f32), vm((2, 256, DM), bf16),
                vm((M, DM), bf16), vm((4, D), bf16), vm((D,), bf16),
                vm((256, 128), bf16), vm((128, 256), bf16),
                vm((2, S, 128), bf16), vm((2, S, 128), bf16), vm((2, 128, S), bf16), vm((2, S, 128), bf16),
                vm((2, 16, 256, 128), f32), vm((2, 16, 256, 128), f32), vm((2, 16, 256, 128), f32),
                vm((256, 128), f32), vm((2, S, 128), bf16), vm((8, D), f32),
                dma((3,)), dma((3,)), dma((5,)), dma, dma((5,)), dma((2,)), dma((2, 3)), dma((2,)), dma((2,))],
            compiler_params=pltpu.CompilerParams(
                vmem_limit_bytes=120 * 1024 * 1024,
                flags={"XLA_TPU_EVENLY_DISTRIBUTE_CRITICAL_NODES": True}),
        )(x.reshape(S, DM), mem0.reshape(M, DM),
          wq.reshape(DM // 2, 2, H, DH), wk.reshape(DM // 2, 2, H, DH), wv.reshape(DM // 2, 2, H, DH),
          wo.reshape(H * DH, DM), q.reshape(S, D), k.reshape(S, D), v.reshape(S, D),
          shift_k.T, ssm_k, ssm_d, jnp.asarray(fwd, bf16), jnp.asarray(inv, bf16))
        return out.reshape(1, S, 2 * D)
    return fn


@jax.jit
def pallas_concat_heads__memory_aug_recurrent_mem_tr__ssm_conv_h3__prompt_kernel(
    A_x, A_mem0, A_Wq, A_Wk, A_Wv, A_Wo, A_seg_len, B_q, B_k, B_v, B_shift_k, B_ssm_k, B_ssm_D,
):
    return make()(A_x, A_mem0, A_Wq, A_Wk, A_Wv, A_Wo, B_q, B_k, B_v, B_shift_k, B_ssm_k, B_ssm_D)
```

```python
import jax
import jax.numpy as jnp
import numpy as np
from jax.experimental import pallas as pl
from jax.experimental.pallas import tpu as pltpu

S, DM, H, DH, M, SEG = 2048, 1024, 32, 128, 8, 32
D = 1024
L = M + SEG
P0 = 512
TS = 24
RING = 576
G = 4
NG = H // G
NB = D // 128
NT = (((1,), (1,)), ((), ()))
NN = (((1,), (0,)), ((), ()))


def _dot(a, b, dims=NN):
    return jax.lax.dot_general(a, b, dims, preferred_element_type=jnp.float32)


def _dft_consts():
    n, c = 256, 128
    f = np.concatenate([np.arange(0, 128, 2), np.arange(1, 128, 2)])
    th = 2 * np.pi * np.outer(f + 0.5, np.arange(c)) / n
    fwd = np.concatenate([np.cos(th), -np.sin(th)], 0)
    inv = np.concatenate([np.cos(th).T, -np.sin(th).T], 1) * (2.0 / n)
    return fwd.astype(np.float32), inv.astype(np.float32)


def _step_plan():
    pre = {0: ["b1", "b1", "b2", "b2", "b2"], 2: ["b2", "b1", "b2", "b2"], 3: ["b1"],
           4: ["b2", "b2"], 7: ["b3"], 8: ["b3"]}
    lag_s, lag_p, split_t, split_g = 1, 3, 10, 5
    plan = []
    for t in range(NG + lag_p):
        if t < NG:
            plan.append(("mm", t))
        if 0 <= t - lag_s < NG:
            g = t - lag_s
            plan += [("qk", g), ("st", g)] if g == NG - 1 else [("st", g), ("qk", g)]
        if 0 <= t - lag_p < NG:
            plan.append(("pv", t - lag_p))
        if t == split_t:
            plan.append(("wo", (0, split_g)))
        plan += [(b, 1) for b in pre.get(t, [])]
    plan.append(("wo", (split_g, NG)))
    return plan


def _kernel(x_hbm, mem0_hbm, wq_hbm, wk_hbm, wv_hbm, wo_hbm,
            q_hbm, k_hbm, v_hbm, sk_hbm, w_hbm, dd_hbm, f_hbm, g_hbm,
            out_hbm,
            xv, raw, wqkv, wo32, ring, osta, mem0v, skv, ddv, fv, gv,
            kin, vin, win, qin, uh, whp, yh, wprev, ost, skt,
            w0sem, wsem, xsem, wosem, smsem, osema, isem, qsem, osem):
    f32, bf16, u32 = jnp.float32, jnp.bfloat16, jnp.uint32

    def in_copies(j, p):
        c = pl.multiple_of(j * 128, 128)
        return [pltpu.make_async_copy(k_hbm.at[:, pl.ds(c, 128)], kin.at[p], isem.at[p, 0]),
                pltpu.make_async_copy(v_hbm.at[:, pl.ds(c, 128)], vin.at[p], isem.at[p, 1]),
                pltpu.make_async_copy(w_hbm.at[pl.ds(c, 128), :], win.at[p], isem.at[p, 2])]

    def q_copy(j, p):
        c = pl.multiple_of(j * 128, 128)
        return pltpu.make_async_copy(q_hbm.at[:, pl.ds(c, 128)], qin.at[p], qsem.at[p])

    def outa_copy(sg, p):
        r = pl.multiple_of(sg * 256, 256)
        return pltpu.make_async_copy(osta.at[p], out_hbm.at[pl.ds(r, 256), pl.ds(0, DM)], osema.at[p])

    def outb_copy(j, p):
        c = pl.multiple_of(D + j * 128, 128)
        return pltpu.make_async_copy(ost.at[p], out_hbm.at[:, pl.ds(c, 128)], osem.at[p])

    wsrc = [w.bitcast(u32) for w in (wq_hbm, wk_hbm, wv_hbm)]

    def w_copies(hp):
        slot = hp % 3
        return [pltpu.make_async_copy(wsrc[j].at[:, par, hp, :], raw.at[slot, 2 * j + par], wsem.at[slot])
                for j in range(3) for par in range(2)]

    def wo_copy(part):
        r = pl.multiple_of(part * 512, 512)
        return pltpu.make_async_copy(wo_hbm.at[pl.ds(r, 512), :],
                                     wo32.bitcast(bf16).at[pl.ds(r, 512), :], wosem)

    def x_copy(part):
        r = pl.multiple_of(part * 512, 512)
        return pltpu.make_async_copy(x_hbm.at[pl.ds(r, 512), :], xv.at[pl.ds(r, 512), :], xsem.at[part + 1])

    small = [pltpu.make_async_copy(a, b, smsem.at[n]) for n, (a, b) in enumerate(
        ((mem0_hbm, mem0v), (sk_hbm, skv), (dd_hbm, ddv), (f_hbm, fv), (g_hbm, gv)))]

    def stage1(j, p, i):
        c0 = pl.multiple_of(j * 128, 128)
        taps = skt[:, pl.ds(c0, 128)]
        dvec = taps[4:5]
        first = i == 0
        prev = jnp.where(first, 0.0, wprev[...])
        kf_prev = None
        for c in range(2):
            rc = pl.multiple_of(i * 256 + c * 128, 128)
            a = 2 * i + c
            kf = kin[p, pl.ds(rc, 128), :].astype(f32)
            if c == 0:
                rp = pl.multiple_of(jnp.maximum(rc - 8, 0), 8)
                tail = jnp.where(first, 0.0, kin[p, pl.ds(rp, 8), :].astype(f32))
            else:
                tail = kf_prev[120:128]
            ext = jnp.concatenate([tail, kf], axis=0)
            ks = (kf * taps[0:1] + ext[7:135] * taps[1:2]
                  + ext[6:134] * taps[2:3] + ext[5:133] * taps[3:4])
            kf_prev = kf
            kv = ks * vin[p, pl.ds(rc, 128), :].astype(f32)
            uh[p, a] = _dot(fv[...], kv)
            yield
            wt = win[p, :, pl.ds(pl.multiple_of(a * 128, 128), 128)]
            wh = _dot(fv[...], wt, NT)
            pr, pi_ = prev[:128], prev[128:]
            re = jnp.concatenate([wh[0:64] - pi_[0:64], wh[64:128] + pi_[64:128]], 0)
            im = jnp.concatenate([wh[128:192] + pr[0:64], wh[192:256] - pr[64:128]], 0)
            if c == 0:
                re = re + jnp.where(first, dvec, 0.0)
            whp[p, a, 0:128] = re
            whp[p, a, 128:256] = im
            prev = wh
            yield
        wprev[...] = prev

    def stage2(p, i):
        ob = 4
        for gg in range(2):
            rr = pl.multiple_of(i * 16 + gg * 8, 8)
            ri = pl.multiple_of(128 + i * 16 + gg * 8, 8)
            for b in range(16 // ob):
                outs = list(range(b * ob, (b + 1) * ob))
                accr, acci, wc = {}, {}, {}
                for ap in range(outs[-1] + 1):
                    ur = uh[p, ap, pl.ds(rr, 8), :]
                    ui = uh[p, ap, pl.ds(ri, 8), :]
                    for a in outs:
                        m = a - ap
                        if m < 0:
                            continue
                        if m not in wc:
                            wc[m] = (whp[p, m, pl.ds(rr, 8), :], whp[p, m, pl.ds(ri, 8), :])
                        wr, wi = wc[m]
                        tr = ur * wr - ui * wi
                        ti = ur * wi + ui * wr
                        accr[a] = tr if a not in accr else accr[a] + tr
                        acci[a] = ti if a not in acci else acci[a] + ti
                for a in outs:
                    yh[p, a, pl.ds(rr, 8), :] = accr[a]
                    yh[p, a, pl.ds(ri, 8), :] = acci[a]
                yield

    def stage3(p, i):
        for c in range(2):
            a = 2 * i + c
            y = _dot(gv[...], yh[p, a])
            r = pl.multiple_of(a * 128, 128)
            ost[p, pl.ds(r, 128), :] = (qin[p, pl.ds(r, 128), :].astype(f32) * y).astype(bf16)
            yield

    def drain(*gens):
        for g in gens:
            for _ in g:
                pass

    def project(hp):
        slot = hp % 3
        lo, hi = [], []
        for j in range(3):
            ev, od = raw[slot, 2 * j], raw[slot, 2 * j + 1]
            lo.append((ev & u32(0xFFFF)) | (od << 16))
            hi.append((ev >> 16) | (od & u32(0xFFFF0000)))
        w32 = jnp.concatenate(lo + hi, axis=1)
        c0 = pl.multiple_of(hp * 768, 768)
        wqkv[:, pl.ds(c0, 768)] = w32
        w = pltpu.bitcast(w32, bf16)
        for rb in range(P0 // 256):
            ring[pl.ds(64 + rb * 256, 256), pl.ds(c0, 768)] = _dot(xv[rb * 256:(rb + 1) * 256, :], w)

    w0 = [[pltpu.make_async_copy(wsrc[j].at[:, par, 0, :], raw.at[0, 2 * j + par], w0sem.at[j]) for par in range(2)]
          for j in range(3)]
    xh = [pltpu.make_async_copy(x_hbm.at[pl.ds(r * 256, 256), :], xv.at[pl.ds(r * 256, 256), :], xsem.at[r])
          for r in range(2)]
    xh[0].start()
    for cp in w0[0]:
        cp.start()
    for cp in small:
        cp.start()
    for cp in w0[1] + w0[2]:
        cp.start()
    xh[1].start()
    yh[1] = jnp.zeros((16, 256, 128), f32)
    qin[1] = jnp.zeros((S, 128), bf16)
    wprev[...] = jnp.zeros((256, 128), f32)
    xh[0].wait()
    first_w = []
    for j in range(3):
        for cp in w0[j]:
            cp.wait()
        ev, od = raw[0, 2 * j], raw[0, 2 * j + 1]
        lo = (ev & u32(0xFFFF)) | (od << 16)
        hi = (ev >> 16) | (od & u32(0xFFFF0000))
        wqkv[:, j * 128:(j + 1) * 128] = lo
        wqkv[:, 384 + j * 128:384 + (j + 1) * 128] = hi
        w = pltpu.bitcast(jnp.concatenate([lo, hi], axis=1), bf16)
        first_w.append(w)
        y = _dot(xv[0:256, :], w)
        ring[64:320, j * 128:(j + 1) * 128] = y[:, :128]
        ring[64:320, 384 + j * 128:384 + (j + 1) * 128] = y[:, 128:]
        if j == 0:
            for cp in w_copies(1):
                cp.start()
    xh[1].wait()
    for j in range(3):
        y = _dot(xv[256:512, :], first_w[j])
        ring[320:576, j * 128:(j + 1) * 128] = y[:, :128]
        ring[320:576, 384 + j * 128:384 + (j + 1) * 128] = y[:, 128:]
    for cp in w_copies(2):
        cp.start()
    for cp in in_copies(0, 0):
        cp.start()
    for cp in small:
        cp.wait()
    skt[0:4, :] = skv[...].astype(f32)
    skt[4:5, :] = ddv[...].astype(f32).reshape(1, D)
    skt[5:8, :] = jnp.zeros((3, D), f32)

    def startup_1(it, carry):
        for cp in w_copies(it):
            cp.wait()
        project(it)
        for cp in w_copies(it + 2):
            cp.start()
        return carry
    startup_1(1, 0)
    for cp in in_copies(0, 0):
        cp.wait()

    def startup_a(it, carry):
        for cp in w_copies(it):
            cp.wait()
        project(it)
        drain(stage1(0, 0, it - 2))
        for cp in w_copies(it + 2):
            cp.start()

        @pl.when(it == 2)
        def _():
            for cp in in_copies(1, 1):
                cp.start()

        @pl.when(it >= 3)
        def _():
            wo_copy(it - 3).start()
        return carry

    def startup_b(it, carry):
        for cp in w_copies(it):
            cp.wait()
        project(it)

        @pl.when(it < 14)
        def _():
            for cp in w_copies(it + 2):
                cp.start()

        @pl.when(it == 10)
        def _():
            wo_copy(7).start()

        @pl.when((it >= 11) & (it < 14))
        def _():
            x_copy(it - 10).start()
        return carry

    jax.lax.fori_loop(2, 10, startup_a, 0)
    jax.lax.fori_loop(10, 16, startup_b, 0)
    for part in range(8):
        wo_copy(part).wait()
    for part in range(1, 4):
        x_copy(part).wait()

    rows = jax.lax.broadcasted_iota(jnp.int32, (L, L), 0)
    cols = jax.lax.broadcasted_iota(jnp.int32, (L, L), 1)
    mask = (rows < M) | (rows >= cols)
    exp_scale = float(DH ** -0.5 * np.log2(np.e))
    neg = -1e9 * DH ** 0.5
    plan = _step_plan()

    def slot_body(sg, mem):
        p = sg % 2

        @pl.when(sg < NB - 1)
        def _():
            for cp in in_copies(sg + 1, 1 - p):
                cp.wait()

        @pl.when(sg >= 1)
        def _():
            q_copy(sg - 1, 1 - p).wait()

        @pl.when(sg < NB - 2)
        def _():
            for cp in in_copies(sg + 2, p):
                cp.start()
        q_copy(sg, p).start()

        @pl.when(sg >= 2)
        def _():
            outa_copy(0, p).wait()

        @pl.when(sg >= 3)
        def _():
            outb_copy(0, 1 - p).wait()

        def step(i, mem):
            s = sg * 8 + i
            xr = pl.multiple_of(P0 + s * TS, 8)
            wr = pl.multiple_of(jax.lax.rem(s * TS, RING), 8)
            rd = pl.multiple_of(jax.lax.rem(s * SEG + 64, RING), 32)
            h = jnp.concatenate([mem, xv[pl.ds(xr, TS), :].astype(f32)], axis=0).astype(bf16)
            gens = {"b1": stage1(jnp.minimum(sg + 1, NB - 1), 1 - p, i),
                    "b2": stage2(p, i),
                    "b3": stage3(1 - p, i)}
            ys, ps, outs, y = {}, {}, {}, None

            def operand(t, ii, j):
                c = ii * 384 + j * 128
                if t == NG - 1 and j < 2:
                    r = ring[pl.ds(rd, SEG), t * G * 384 + c:t * G * 384 + c + 128]
                    y = ys[t][:, c:c + 128]
                    y0, y1, y2 = y[8:16], y[16:24], y[24:32]
                    g1 = jnp.where(s == 63, y0, r[8:16])
                    g2 = jnp.where(s == 62, y0, jnp.where(s == 63, y1, r[16:24]))
                    g3 = jnp.where(s == 61, y0, jnp.where(s == 62, y1, jnp.where(s == 63, y2, r[24:32])))
                    return jnp.concatenate([y[:M], r[0:8], g1, g2, g3], 0)
                return jnp.concatenate(
                    [ys[t][:M, c:c + 128], ring[pl.ds(rd, SEG), t * G * 384 + c:t * G * 384 + c + 128]], 0)

            for op, t in plan:
                if op == "mm":
                    ys[t] = _dot(h, pltpu.bitcast(wqkv[:, t * G * 384:(t + 1) * G * 384], bf16))
                elif op == "st":
                    ring[pl.ds(wr, TS), t * G * 384:(t + 1) * G * 384] = ys[t][M:, :]
                elif op == "qk":
                    ps[t] = []
                    for ii in range(G):
                        sc = jnp.where(mask, _dot(operand(t, ii, 0), operand(t, ii, 1), NT), neg)
                        e = jnp.exp2((sc - jnp.max(sc, axis=1, keepdims=True)) * exp_scale)
                        l = jnp.sum(e, axis=1, keepdims=True)
                        r = pltpu.reciprocal(l, approx=True)
                        ps[t].append((e, r * (2.0 - l * r)))
                elif op == "pv":
                    outs[t] = [_dot(ps[t][ii][0], operand(t, ii, 2)) * ps[t][ii][1] for ii in range(G)]
                elif op == "wo":
                    t0, t1 = t
                    o = jnp.concatenate([oo for tt in range(t0, t1) for oo in outs[tt]], axis=1)
                    yy = _dot(o, pltpu.bitcast(wo32[t0 * G * 64:t1 * G * 64, :], bf16))
                    y = yy if y is None else y + yy
                else:
                    next(gens[op], None)
            drain(*gens.values())
            osta[p, pl.ds(pl.multiple_of(i * SEG, SEG), SEG), :] = y[M:, :].astype(bf16)
            return y[:M, :]

        mem = jax.lax.fori_loop(0, 8, step, mem, unroll=4)
        outa_copy(sg, p).start()

        @pl.when(sg >= 1)
        def _():
            outb_copy(sg - 1, 1 - p).start()
        return mem

    jax.lax.fori_loop(0, NB, slot_body, mem0v[...].astype(f32))

    jl = NB - 1
    q_copy(jl, jl % 2).wait()
    outb_copy(0, jl % 2).wait()

    def last_copy(i):
        r = pl.multiple_of(i * 256, 256)
        return pltpu.make_async_copy(ost.at[jl % 2, pl.ds(r, 256), :],
                                     out_hbm.at[pl.ds(r, 256), pl.ds(D + jl * 128, 128)], osem.at[jl % 2])

    def epilogue(i, carry):
        drain(stage3(jl % 2, i))
        last_copy(i).start()
        return carry
    jax.lax.fori_loop(0, 8, epilogue, 0)
    for p in range(2):
        outa_copy(0, p).wait()
    outb_copy(0, 1 - jl % 2).wait()
    for i in range(8):
        last_copy(i).wait()


def make():
    def fn(x, mem0, wq, wk, wv, wo, q, k, v, shift_k, ssm_k, ssm_d):
        fwd, inv = _dft_consts()
        any_ = pl.BlockSpec(memory_space=pl.ANY)
        vm, dma = pltpu.VMEM, pltpu.SemaphoreType.DMA
        f32, bf16, u32 = jnp.float32, jnp.bfloat16, jnp.uint32
        out = pl.pallas_call(
            _kernel,
            out_shape=jax.ShapeDtypeStruct((S, 2 * D), bf16),
            in_specs=[any_] * 14,
            out_specs=any_,
            scratch_shapes=[
                vm((S, DM), bf16), vm((3, 6, DM // 2, 128), u32),
                vm((DM // 2, H * 384), u32), vm((H * DH // 2, DM), u32),
                vm((RING, H * 384), f32), vm((2, 256, DM), bf16),
                vm((M, DM), bf16), vm((4, D), bf16), vm((D,), bf16),
                vm((256, 128), bf16), vm((128, 256), bf16),
                vm((2, S, 128), bf16), vm((2, S, 128), bf16), vm((2, 128, S), bf16), vm((2, S, 128), bf16),
                vm((2, 16, 256, 128), f32), vm((2, 16, 256, 128), f32), vm((2, 16, 256, 128), f32),
                vm((256, 128), f32), vm((2, S, 128), bf16), vm((8, D), f32),
                dma((3,)), dma((3,)), dma((5,)), dma, dma((5,)), dma((2,)), dma((2, 3)), dma((2,)), dma((2,))],
            compiler_params=pltpu.CompilerParams(
                vmem_limit_bytes=120 * 1024 * 1024,
                flags={"XLA_TPU_EVENLY_DISTRIBUTE_CRITICAL_NODES": True}),
        )(x.reshape(S, DM), mem0.reshape(M, DM),
          wq.reshape(DM // 2, 2, H, DH), wk.reshape(DM // 2, 2, H, DH), wv.reshape(DM // 2, 2, H, DH),
          wo.reshape(H * DH, DM), q.reshape(S, D), k.reshape(S, D), v.reshape(S, D),
          shift_k.T, ssm_k, ssm_d, jnp.asarray(fwd, bf16), jnp.asarray(inv, bf16))
        return out.reshape(1, S, 2 * D)
    return fn


@jax.jit
def pallas_concat_heads__memory_aug_recurrent_mem_tr__ssm_conv_h3__prompt_kernel(
    A_x, A_mem0, A_Wq, A_Wk, A_Wv, A_Wo, A_seg_len, B_q, B_k, B_v, B_shift_k, B_ssm_k, B_ssm_D,
):
    return make()(A_x, A_mem0, A_Wq, A_Wk, A_Wv, A_Wo, B_q, B_k, B_v, B_shift_k, B_ssm_k, B_ssm_D)
```
